```python
import os as _os
_os.environ.setdefault('JAX_PLATFORMS', 'cpu')
import jax
import jax.numpy as jnp

def _softmax(x, axis=-1):
    return jax.nn.softmax(x, axis=axis)

def _gelu(x):
    return jax.nn.gelu(x, approximate=True)

def _silu(x):
    return jax.nn.silu(x)

def _sigmoid(x):
    return jax.nn.sigmoid(x)

def _layernorm(x, axis=-1, eps=1e-05):
    m = jnp.mean(x, axis=axis, keepdims=True)
    v = jnp.var(x, axis=axis, keepdims=True)
    return (x - m) / jnp.sqrt(v + eps)

def _scatter_add(tgt, idx, src, axis=0):
    return tgt.at[idx].add(src)

def _segment_sum(src, seg, n):
    return jax.ops.segment_sum(src, seg, n)

class _Rng:

    def __init__(self, key):
        self._k = key

    def _next(self):
        self._k, sub = jax.random.split(self._k)
        return sub

    def normal(self, shape):
        return jax.random.normal(self._next(), shape, dtype=jnp.bfloat16)

    def randint(self, lo, hi, shape):
        return jax.random.randint(self._next(), shape, lo, hi, dtype=jnp.int32)

    def uniform(self, shape, lo=0.0, hi=1.0):
        return jax.random.uniform(self._next(), shape, jnp.bfloat16, lo, hi)

    def permutation(self, n):
        return jax.random.permutation(self._next(), n)
kernel_name = 'gated_mix__grouped_kv_mqa__memory_aug_recurrent_mem_tr__prompt'

def setup_inputs():
    _rng = _Rng(jax.random.key(int.from_bytes(__import__("os").urandom(4), "little")))
    _w = lambda a: (lambda t: t.astype(jnp.bfloat16) if jnp.issubdtype(t.dtype, jnp.floating) else t)(jnp.asarray(a))

    def _A_setup():
        B, S, D, H = (1, 2048, 1024, 32)
        Dh = D // H
        return {'x': _w((lambda *s: _rng.normal(s) * 0.05)(B, S, D)), 'wq': _w((lambda *s: _rng.normal(s) * 1.6)(D, H * Dh)), 'wk': _w((lambda *s: _rng.normal(s) * 1.6)(D, Dh)), 'wv': _w((lambda *s: _rng.normal(s) * 0.05)(D, Dh)), 'wo': _w((lambda *s: _rng.normal(s) * 0.05)(H * Dh, D))}
    _A_in = _A_setup()

    def _B_setup():
        B, S, Dm = (1, 2048, 1024)
        H, Dh = (32, 128)
        M, seg = (8, 32)
        seg = min(seg, S)
        S = S // seg * seg
        return {'x': _w((lambda *s: _rng.normal(s) * 0.05)(B, S, Dm)), 'mem0': _w((lambda *s: _rng.normal(s) * 0.8)(B, M, Dm)), 'Wq': _w((lambda *s: _rng.normal(s) * 3.2)(Dm, H, Dh) * Dm ** (-0.5)), 'Wk': _w((lambda *s: _rng.normal(s) * 3.2)(Dm, H, Dh) * Dm ** (-0.5)), 'Wv': _w((lambda *s: _rng.normal(s) * 0.8)(Dm, H, Dh) * Dm ** (-0.5)), 'Wo': _w((lambda *s: _rng.normal(s) * 0.8)(H, Dh, Dm) * (H * Dh) ** (-0.5)), 'seg_len': seg}
    _B_in = _B_setup()
    return {'A_x': _A_in['x'], 'A_wq': _A_in['wq'], 'A_wk': _A_in['wk'], 'A_wv': _A_in['wv'], 'A_wo': _A_in['wo'], 'B_x': _B_in['x'], 'B_mem0': _B_in['mem0'], 'B_Wq': _B_in['Wq'], 'B_Wk': _B_in['Wk'], 'B_Wv': _B_in['Wv'], 'B_Wo': _B_in['Wo'], 'B_seg_len': _B_in['seg_len'], 'gate_w': _w((lambda *s: _rng.normal(s) * 0.05)(1024) * 16.0)}

def reference(A_x, A_wq, A_wk, A_wv, A_wo, B_x, B_mem0, B_Wq, B_Wk, B_Wv, B_Wo, B_seg_len, gate_w):

    def _A_ref(x, wq, wk, wv, wo):
        B, S, D = x.shape
        H = 32
        Dh = D // H
        q = (lambda x, *d: x.transpose(*d))((x @ wq).reshape(B, S, H, Dh), 0, 2, 1, 3)
        k = x @ wk
        v = x @ wv
        scores = jnp.einsum('bhqd,bkd->bhqk', q, k) * Dh ** (-0.5)
        p = _softmax(scores, axis=-1)
        o = jnp.einsum('bhqk,bkd->bhqd', p, v)
        return (lambda x, *d: x.transpose(*d))(o, 0, 2, 1, 3).reshape(B, S, H * Dh) @ wo

    def _B_ref(x, mem0, Wq, Wk, Wv, Wo, seg_len):
        B, S, Dm = x.shape
        H, Dh = (Wq.shape[1], Wq.shape[2])
        M = mem0.shape[1]
        scale = Dh ** (-0.5)
        n_seg = S // seg_len
        L = M + seg_len
        idx = jnp.arange(L)
        mask = (idx[:, None] < M) | (idx[:, None] >= idx[None, :])
        mem = mem0
        outs = []
        for s in range(n_seg):
            xs = x[:, s * seg_len:(s + 1) * seg_len, :].copy()
            h = jnp.concatenate([mem, xs], axis=1)
            q = jnp.einsum('btd,dhe->bhte', h, Wq)
            k = jnp.einsum('btd,dhe->bhte', h, Wk)
            v = jnp.einsum('btd,dhe->bhte', h, Wv)
            scores = jnp.einsum('bhqe,bhke->bhqk', q, k) * scale
            scores = jnp.where(mask[None, None], scores, -1000000000.0)
            p = _softmax(scores, axis=-1)
            o = jnp.einsum('bhqk,bhke->bhqe', p, v)
            o = jnp.einsum('bhte,hed->btd', o, Wo)
            mem = o[:, :M, :].copy()
            outs.append(o[:, M:, :])
        return jnp.concatenate(outs, axis=1)
    x = A_x
    g = _sigmoid((x * gate_w).sum(-1, keepdims=True))
    a = _A_ref(x, A_wq, A_wk, A_wv, A_wo)
    b = _B_ref(x, B_mem0, B_Wq, B_Wk, B_Wv, B_Wo, B_seg_len)
    return g * a + (1 - g) * b
```

```python
import functools
import jax
import jax.numpy as jnp
import numpy as np
from jax import lax
import jax.experimental.pallas as pl
import jax.experimental.pallas.tpu as pltpu

BF = jnp.bfloat16
F32 = jnp.float32
U32 = jnp.uint32

S = 2048
D = 1024
HA, DA = 32, 32
HB, DB = 32, 128
LOG2E = 1.4426950408889634
SCALE_A = float(np.asarray(DA ** -0.5, dtype=BF)) * LOG2E
SCALE_B = float(np.asarray(DB ** -0.5, dtype=BF)) * LOG2E
NEG = -1e30

XB = 256
NXB = S // XB
NQT = S // 128
NUNITS = NQT * (HA // 4)
NC = S // 128
SKEW = 2
OB = 256


def build(cfg):
    do_a = cfg.get('a', True); do_b = cfg.get('b', True); do_rel = cfg.get('rel', True)
    do_proj = cfg.get('proj', True); do_epi = cfg.get('epi', True)
    UA = cfg.get('UA', 4)
    UF = cfg.get('UF', 2)
    NPAIR = S // 64
    NU_F = UF * NPAIR
    NU_S = NUNITS - NU_F
    NIT_S = NU_S // UA
    L1, L2 = cfg.get('L1', 1), cfg.get('L2', 2)

    def kernel(x_hbm, wq_hbm, wk_ref, wv_ref, wo_hbm, mem0_ref, bq_hbm, bk_hbm, bv_hbm, bo_hbm, gw_ref,
               out_hbm,
               x_v, wq_v, wo_v, raw_v, wp_v, bo_v, qt_v, k_v, vt_v, sa_v, sb_v, o_v, b_v, sv_v, so_v, ob_v,
               xsem, wsem, bosem, osem):
        sbuf = (sa_v, sb_v)

        def x_copy(i):
            return pltpu.make_async_copy(x_hbm.at[pl.ds(i * XB, XB)], x_v.at[pl.ds(i * XB, XB)], xsem.at[i])
        wq_copy = pltpu.make_async_copy(wq_hbm, wq_v, wsem.at[0])
        wo_copy = pltpu.make_async_copy(wo_hbm, wo_v, wsem.at[1])
        raw_copies = [pltpu.make_async_copy(src, raw_v.at[m], wsem.at[2 + m])
                      for m, src in enumerate((bq_hbm, bk_hbm, bv_hbm))]
        bo_copies = [pltpu.make_async_copy(bo_hbm.at[:, pl.ds(n * 128, 128)], bo_v.at[n], bosem.at[n])
                     for n in range(8)]

        wq_copy.start()
        for i in range(NXB):
            x_copy(i).start()
        wq_copy.wait()
        for c in raw_copies:
            c.start()
        for c in bo_copies:
            c.start()
        wo_copy.start()

        wkv = jnp.concatenate([wk_ref[...], wv_ref[...], jnp.zeros((D, 64), BF)], axis=1)

        def proj_body(rb, carry):
            x_copy(rb).wait()
            if do_proj:
                r0 = pl.multiple_of(rb * XB, XB)
                xb = x_v[pl.ds(r0, XB), :]
                kv = jnp.dot(xb, wkv, preferred_element_type=F32)
                k_v[pl.ds(r0, XB), :] = kv[:, :DA].astype(BF)
                kvt = kv.T
                q = jnp.dot(xb, wq_v[...], preferred_element_type=F32) * SCALE_A
                qt = q.T
                for t in range(XB // 128):
                    vt_v[rb * (XB // 128) + t] = kvt[DA:2 * DA, t * 128:(t + 1) * 128].astype(BF)
                    qt_v[rb * (XB // 128) + t] = qt[:, t * 128:(t + 1) * 128].astype(BF)
            return carry
        lax.fori_loop(0, NXB, proj_body, 0)

        def load_q(u):
            u = jnp.minimum(u, NUNITS - 1)
            qi = u // 8
            g = u % 8
            base = pl.multiple_of(g * 128, 128)
            return jnp.concatenate(
                [qt_v[qi, pl.ds(base + 32 * j, 32), :] for j in range(4)], axis=1)

        def qk_chunk(qt, s_ref, c, m8):
            sn = jnp.dot(k_v[c * 128:(c + 1) * 128, :], qt, preferred_element_type=F32)
            s_ref[c * 128:(c + 1) * 128, :] = sn
            for g in range(16):
                t = sn[g * 8:(g + 1) * 8]
                m8 = t if m8 is None else jnp.maximum(m8, t)
            return m8

        class AState:
            pass

        def a_tasks(u0, nu, st):
            tasks = []
            def mk(k, c):
                def run():
                    if c == 0:
                        st.mc8 = jnp.broadcast_to(st.m, (8, 512))
                        st.l8 = None
                        st.acc = None
                        st.hist = []
                    cn = c + SKEW
                    if cn < NC:
                        if c == 0:
                            st.qt = load_q(u0 + k + 1)
                        st.m8 = qk_chunk(st.qt, sbuf[(k + 1) % 2], cn, st.m8)
                        if cn == NC - 1:
                            st.mnext = jnp.max(st.m8, axis=0, keepdims=True)
                    else:
                        if cn == NC:
                            st.qt = load_q(u0 + k + 2)
                            st.m8 = None
                        st.m8 = qk_chunk(st.qt, sbuf[k % 2], cn - NC, st.m8)
                    st.hist.append(st.m8)
                    me = st.mc8
                    if st.l8 is not None:
                        me = me + st.l8 * 0.0
                    if c >= 2:
                        me = me + st.hist[c - 2] * 0.0
                    sc = sbuf[k % 2][c * 128:(c + 1) * 128, :].reshape(16, 8, 512)
                    p = jnp.exp2(sc - me[None])
                    l8 = st.l8
                    for g in reversed(range(16)):
                        l8 = p[g] if l8 is None else l8 + p[g]
                    st.l8 = l8
                    pv = jnp.dot(vt_v[c], p.reshape(128, 512).astype(BF), preferred_element_type=F32)
                    st.acc = pv if st.acc is None else st.acc + pv
                    if c == NC - 1:
                        l = jnp.sum(st.l8, axis=0, keepdims=True)
                        o = st.acc * (1.0 / l)
                        o4 = jnp.concatenate([o[:, j * 128:(j + 1) * 128] for j in range(4)], axis=0)
                        u = u0 + k
                        o_v[u % 8, pl.ds(pl.multiple_of((u // 8) * 128, 128), 128), :] = o4.T.astype(BF)
                        st.m = st.mnext
                return run
            for k in range(nu):
                for c in range(NC):
                    tasks.append(mk(k, c))
            return tasks

        def relayout_block(blk):
            m = blk // 64
            i = blk % 64
            w = raw_v[m, pl.ds(pl.multiple_of(i * 16, 16), 16)]
            evs, ods = [], []
            for t in range(8):
                a = pltpu.bitcast(w[2 * t], U32)
                b = pltpu.bitcast(w[2 * t + 1], U32)
                evs.append((a & jnp.uint32(0xFFFF)) | (b << 16))
                ods.append((a >> 16) | (b & jnp.uint32(0xFFFF0000)))
            ev = jnp.swapaxes(jnp.stack(evs), 0, 1)
            od = jnp.swapaxes(jnp.stack(ods), 0, 1)
            r0 = pl.multiple_of(i * 8, 8)
            for j in range(16):
                wp_v[m, 2 * j, pl.ds(r0, 8), :] = ev[j]
                wp_v[m, 2 * j + 1, pl.ds(r0, 8), :] = od[j]

        if do_a:
            qt0 = load_q(0)
            m8 = None
            for c in range(NC):
                m8 = qk_chunk(qt0, sa_v, c, m8)
            m_init = jnp.max(m8, axis=0, keepdims=True)
            qt1 = load_q(1)
            m8 = None
            for c in range(SKEW):
                m8 = qk_chunk(qt1, sb_v, c, m8)
            m8_init = m8
        else:
            m_init = jnp.zeros((1, 512), F32); m8_init = jnp.zeros((8, 512), F32)

        RPI = 192 // NIT_S

        def sa_body(it, carry):
            for m in range(3):
                first = (64 * m) // RPI
                @pl.when(it == first)
                def _():
                    raw_copies[m].wait()
            st = AState()
            st.m, st.m8 = carry
            tasks = a_tasks(it * UA, UA, st) if do_a else []
            nt = max(len(tasks), RPI)
            rel_at = {(r * nt) // RPI: r for r in range(RPI)}
            for n in range(nt):
                if n < len(tasks):
                    tasks[n]()
                if n in rel_at and do_rel:
                    relayout_block(it * RPI + rel_at[n])
            return st.m, st.m8
        carry_a = lax.fori_loop(0, NIT_S, sa_body, (m_init, m8_init))

        for c in bo_copies:
            c.wait()

        r = lax.broadcasted_iota(jnp.int32, (48, 48), 0)
        cc = lax.broadcasted_iota(jnp.int32, (48, 48), 1)
        mask_e = (cc >= 40) | ((cc < 32) & (cc <= r))
        kpos = jnp.where(cc < 24, cc + 8, jnp.where(cc < 32, -1, jnp.where(cc < 40, cc - 32, 1000)))
        qpos = jnp.where(r < 24, r + 8, jnp.where(r < 32, 100, r - 32))
        mask_o = kpos <= qpos

        def b_step(lhs, even, base, filler):
            mask = mask_e if even else mask_o
            qkv, ps, os_ = {}, {}, {}
            def wmat(m, h):
                return pltpu.bitcast(wp_v[m, h], BF)
            def do_qkv(h):
                q = (jnp.dot(lhs, wmat(0, h), preferred_element_type=F32) * SCALE_B).astype(BF)
                k = jnp.dot(lhs, wmat(1, h), preferred_element_type=F32).astype(BF)
                v = jnp.dot(lhs, wmat(2, h), preferred_element_type=F32).astype(BF)
                if even:
                    sv_v[3 * h] = q[32:48]; sv_v[3 * h + 1] = k[32:48]; sv_v[3 * h + 2] = v[32:48]
                else:
                    q = jnp.concatenate([q, sv_v[3 * h]], axis=0)
                    k = jnp.concatenate([k, sv_v[3 * h + 1]], axis=0)
                    v = jnp.concatenate([v, sv_v[3 * h + 2]], axis=0)
                qkv[h] = (q, k, v)
            def do_s(h):
                q, k, _ = qkv[h]
                s = lax.dot_general(q, k, (((1,), (1,)), ((), ())), preferred_element_type=F32)
                s = jnp.where(mask, s, NEG)
                m = jnp.max(s, axis=-1, keepdims=True)
                p = jnp.exp2(s - m)
                l = jnp.sum(p, axis=-1, keepdims=True)
                ps[h] = (p * pl.reciprocal(l, approx=True)).astype(BF)
            def do_pv(h):
                o = jnp.dot(ps[h], qkv[h][2], preferred_element_type=F32)
                if even:
                    so_v[h] = o[24:32]
                    os_[h] = jnp.concatenate([o[0:24], o[40:48]], axis=0).astype(BF)
                else:
                    os_[h] = jnp.concatenate([o[0:40], so_v[h]], axis=0).astype(BF)
            for h in range(HB + L1 + L2):
                if h < HB:
                    do_qkv(h)
                if 0 <= h - L1 < HB:
                    do_s(h - L1)
                if 0 <= h - L1 - L2 < HB:
                    do_pv(h - L1 - L2)
                filler('head', h)
            ol = jnp.concatenate([os_[h] for h in range(HB)], axis=1)
            ms = []
            for n in range(8):
                y = jnp.dot(ol, bo_v[n], preferred_element_type=F32)
                cols = slice(n * 128, (n + 1) * 128)
                if even:
                    b_v[pl.ds(base, 24), cols] = y[0:24]
                else:
                    b_v[pl.ds(base + 40, 24), cols] = y[0:24]
                    b_v[pl.ds(base + 32, 8), cols] = y[32:40]
                    b_v[pl.ds(base + 24, 8), cols] = y[40:48]
                ms.append(y[24:32].astype(BF))
                filler('wo', n)
            return jnp.concatenate(ms, axis=1)

        per_step = NC * UF // 2
        slots = cfg.get('slots')
        if slots is None:
            slots = {('head', HB): 1, ('head', HB + 1): 1, ('head', HB + 2): 1, ('wo', 7): 2}
            rest = per_step - sum(slots.values())
            for t in range(rest):
                key = ('head', (t * HB) // rest + 1)
                slots[key] = slots.get(key, 0) + 1
        assert sum(slots.values()) == per_step

        def fused_body(t, carry):
            mem, m, m8 = carry
            st = AState()
            st.m, st.m8 = m, m8
            tasks = a_tasks(NU_S + t * UF, UF, st) if (do_a and UF) else []
            it = iter(tasks)
            def filler(kind, idx):
                for _ in range(slots.get((kind, idx), 0)):
                    task = next(it, None)
                    if task is not None:
                        task()
            if do_b:
                base = pl.multiple_of(t * 64, 64)
                mem = b_step(jnp.concatenate([x_v[pl.ds(base, 40), :], mem], axis=0), True, base, filler)
                mem = b_step(jnp.concatenate([x_v[pl.ds(base + 40, 24), :], mem], axis=0), False, base, filler)
            for task in it:
                task()
            return mem, st.m, st.m8
        lax.fori_loop(0, NPAIR, fused_body, (mem0_ref[...], carry_a[0], carry_a[1]))

        wo_copy.wait()
        gw = gw_ref[...].astype(F32)

        def out_copy(i, slot):
            return pltpu.make_async_copy(ob_v.at[slot], out_hbm.at[pl.ds(i * OB, OB)], osem.at[slot])

        def epi_body(i, carry):
            slot = i % 2
            r0 = pl.multiple_of(i * OB, OB)
            @pl.when(i >= 2)
            def _():
                out_copy(i - 2, slot).wait()
            if do_epi:
                ol = jnp.concatenate([o_v[g, pl.ds(r0, OB), :] for g in range(8)], axis=1)
                a = jnp.dot(ol, wo_v[...], preferred_element_type=F32)
                logit = jnp.sum(x_v[pl.ds(r0, OB), :].astype(F32) * gw, axis=-1, keepdims=True)
                g_ = jax.nn.sigmoid(logit)
                bb = b_v[pl.ds(r0, OB), :]
                ob_v[slot] = (g_ * a + (1.0 - g_) * bb).astype(BF)
            else:
                ob_v[slot] = x_v[pl.ds(r0, OB), :]
            out_copy(i, slot).start()
            return carry
        lax.fori_loop(0, S // OB, epi_body, 0)
        out_copy(S // OB - 2, 0).wait()
        out_copy(S // OB - 1, 1).wait()

    def fn(A_x, A_wq, A_wk, A_wv, A_wo, B_x, B_mem0, B_Wq, B_Wk, B_Wv, B_Wo, B_seg_len, gate_w):
        any_spec = pl.BlockSpec(memory_space=pl.ANY)
        vmem_spec = pl.BlockSpec(memory_space=pltpu.VMEM)
        out = pl.pallas_call(
            kernel,
            out_shape=jax.ShapeDtypeStruct((S, D), BF),
            in_specs=[any_spec, any_spec, vmem_spec, vmem_spec, any_spec, vmem_spec,
                      any_spec, any_spec, any_spec, any_spec, vmem_spec],
            out_specs=any_spec,
            scratch_shapes=[
                pltpu.VMEM((S, D), BF),
                pltpu.VMEM((D, D), BF),
                pltpu.VMEM((D, D), BF),
                pltpu.VMEM((3, D, HB, DB), BF),
                pltpu.VMEM((3, HB, D // 2, DB), U32),
                pltpu.VMEM((8, HB * DB, 128), BF),
                pltpu.VMEM((NQT, D, 128), BF),
                pltpu.VMEM((S, DA), BF),
                pltpu.VMEM((NC, DA, 128), BF),
                pltpu.VMEM((S, 512), F32),
                pltpu.VMEM((S, 512), F32),
                pltpu.VMEM((8, S, 128), BF),
                pltpu.VMEM((S, D), F32),
                pltpu.VMEM((3 * HB, 16, DB), BF),
                pltpu.VMEM((HB, 8, DB), F32),
                pltpu.VMEM((2, OB, D), BF),
                pltpu.SemaphoreType.DMA((NXB,)),
                pltpu.SemaphoreType.DMA((5,)),
                pltpu.SemaphoreType.DMA((8,)),
                pltpu.SemaphoreType.DMA((2,)),
            ],
            compiler_params=pltpu.CompilerParams(vmem_limit_bytes=120 * 1024 * 1024),
        )(A_x.reshape(S, D), A_wq, A_wk, A_wv, A_wo, B_mem0.reshape(8, D), B_Wq, B_Wk, B_Wv,
          B_Wo.reshape(HB * DB, D), gate_w.reshape(1, D))
        return out.reshape(1, S, D)
    return jax.jit(fn)


_FN = build({})


@jax.jit
def pallas_gated_mix__grouped_kv_mqa__memory_aug_recurrent_mem_tr__prompt_kernel(
    A_x: jax.Array,
    A_wq: jax.Array,
    A_wk: jax.Array,
    A_wv: jax.Array,
    A_wo: jax.Array,
    B_x: jax.Array,
    B_mem0: jax.Array,
    B_Wq: jax.Array,
    B_Wk: jax.Array,
    B_Wv: jax.Array,
    B_Wo: jax.Array,
    B_seg_len: jax.Array,
    gate_w: jax.Array,
):
    return _FN(A_x, A_wq, A_wk, A_wv, A_wo, B_x, B_mem0, B_Wq, B_Wk, B_Wv, B_Wo, B_seg_len, gate_w)
```

```python
import functools
import jax
import jax.numpy as jnp
import numpy as np
from jax import lax
import jax.experimental.pallas as pl
import jax.experimental.pallas.tpu as pltpu

BF = jnp.bfloat16
F32 = jnp.float32
U32 = jnp.uint32

S = 2048
D = 1024
HA, DA = 32, 32
HB, DB = 32, 128
LOG2E = 1.4426950408889634
SCALE_A = float(np.asarray(DA ** -0.5, dtype=BF)) * LOG2E
SCALE_B = float(np.asarray(DB ** -0.5, dtype=BF)) * LOG2E
NEG = -1e30

XB = 256
NXB = S // XB
NQT = S // 128
NUNITS = NQT * (HA // 4)
NC = S // 128
OB = 256
NT = (((1,), (1,)), ((), ()))


def build(cfg):
    do_a = cfg.get('a', True); do_b = cfg.get('b', True); do_rel = cfg.get('rel', True)
    UA = cfg.get('UA', 4)
    PPI = cfg.get('PPI', 1)
    UF = cfg.get('UF', 2)
    SKEW = cfg.get('SKEW', 2)
    LAGM = cfg.get('LAGM', 2)
    FIN = cfg.get('FIN', 2)
    NPAIR = S // 64
    NIT_F = NPAIR // PPI
    NU_F = UF * NIT_F
    NU_S = NUNITS - NU_F
    NIT_S = NU_S // UA
    L1, L2 = cfg.get('L1', 1), cfg.get('L2', 2)
    assert UA % 2 == 0 and UF % 2 == 0 and NU_S % UA == 0 and 192 % NIT_S == 0

    def kernel(x_hbm, wq_hbm, wkt_hbm, wvt_hbm, wo_hbm, mem0_hbm, bq_hbm, bk_hbm, bv_hbm, bo_hbm, gw_hbm,
               out_hbm,
               x_v, wq_v, wo_v, wkv_v, mem0_v, gw_v, raw_v, wp_v, bo_v, qt_v, k_v, vt_v, sa_v, sb_v, o_v, b_v,
               sq_v, skv_v, ob_v,
               xsem, wqsem, wsem, bosem, osem):
        sbuf = (sa_v, sb_v)

        def x_copy(i):
            return pltpu.make_async_copy(x_hbm.at[pl.ds(i * XB, XB)], x_v.at[pl.ds(i * XB, XB)], xsem.at[i])
        wq_copies = [pltpu.make_async_copy(wq_hbm.at[:, pl.ds(n * 256, 256)], wq_v.at[n], wqsem.at[n])
                     for n in range(4)]
        wo_copy = pltpu.make_async_copy(wo_hbm, wo_v, wsem.at[0])
        raw_copies = [pltpu.make_async_copy(src, raw_v.at[m], wsem.at[1 + m])
                      for m, src in enumerate((bq_hbm, bk_hbm, bv_hbm))]
        wk_copy = pltpu.make_async_copy(wkt_hbm, wkv_v.at[pl.ds(0, DA)], wsem.at[4])
        wv_copy = pltpu.make_async_copy(wvt_hbm, wkv_v.at[pl.ds(DA, DA)], wsem.at[5])
        mem_copy = pltpu.make_async_copy(mem0_hbm, mem0_v, wsem.at[6])
        gw_copy = pltpu.make_async_copy(gw_hbm, gw_v, wsem.at[7])
        bo_copies = [pltpu.make_async_copy(bo_hbm.at[:, pl.ds(n * 128, 128)], bo_v.at[n], bosem.at[n])
                     for n in range(8)]

        wk_copy.start()
        wv_copy.start()
        x_copy(0).start()
        for c in wq_copies:
            c.start()

        def proj_block(rb, first):
            r0 = rb * XB if first else pl.multiple_of(rb * XB, XB)
            x_copy(rb).wait()
            if first:
                wk_copy.wait()
                wv_copy.wait()
            xb = x_v[pl.ds(r0, XB), :]
            kvt = lax.dot_general(wkv_v[...], xb, NT, preferred_element_type=F32)
            k_v[pl.ds(r0, XB), :] = kvt[:DA].T.astype(BF)
            for t in range(XB // 128):
                vt_v[rb * (XB // 128) + t] = kvt[DA:2 * DA, t * 128:(t + 1) * 128].astype(BF)
            for n in range(4):
                if first:
                    wq_copies[n].wait()
                    if n == 1:
                        for i in range(1, NXB):
                            x_copy(i).start()
                    if n == 3:
                        for c in raw_copies + bo_copies + [wo_copy, mem_copy, gw_copy]:
                            c.start()
                q = jnp.dot(xb, wq_v[n], preferred_element_type=F32) * SCALE_A
                qt = q.T
                for t in range(XB // 128):
                    qt_v[rb * (XB // 128) + t, n * 256:(n + 1) * 256, :] = qt[:, t * 128:(t + 1) * 128].astype(BF)

        with jax.named_scope('P1_proj'):
            proj_block(0, True)
            def proj_body(rb, carry):
                proj_block(rb, False)
                return carry
            lax.fori_loop(1, NXB, proj_body, 0)

        def load_q(u):
            u = jnp.minimum(u, NUNITS - 1)
            qi = lax.shift_right_logical(u, 3)
            base = pl.multiple_of((u & 7) * 128, 128)
            return jnp.concatenate(
                [qt_v[qi, pl.ds(base + 32 * j, 32), :] for j in range(4)], axis=1)

        def qk_chunk(qt, s_ref, c, m8):
            sn = jnp.dot(k_v[c * 128:(c + 1) * 128, :], qt, preferred_element_type=F32)
            s_ref[c * 128:(c + 1) * 128, :] = sn
            for g in range(16):
                t = sn[g * 8:(g + 1) * 8]
                m8 = t if m8 is None else jnp.maximum(m8, t)
            return m8

        def finalize(u, acc, l8):
            u = jnp.maximum(u, 0)
            l = jnp.sum(l8, axis=0, keepdims=True)
            inv = pl.reciprocal(l, approx=True)
            inv = inv * (2.0 - l * inv)
            o = acc * inv
            o4 = jnp.concatenate([o[:, j * 128:(j + 1) * 128] for j in range(4)], axis=0)
            row = pl.multiple_of(lax.shift_right_logical(u, 3) * 128, 128)
            o_v[u & 7, pl.ds(row, 128), :] = o4.T.astype(BF)

        class AState:
            pass

        def a_state(carry):
            st = AState()
            st.m, st.m8, st.pacc, st.pl8 = carry
            st.anchor = None
            st.hist = []
            return st

        def a_carry(st):
            return st.m, st.m8, st.pacc, st.pl8

        def a_tasks(u0, nu, st):
            tasks = []
            def mk(k, c):
                def run():
                    if c == 0:
                        st.mc8 = jnp.broadcast_to(st.m, (8, 512))
                        st.l8 = None
                        st.acc = None
                    cn = c + SKEW
                    if cn < NC:
                        if c == 0 and k == 0:
                            st.qt = load_q(u0 + k + 1)
                        st.m8 = qk_chunk(st.qt, sbuf[(k + 1) % 2], cn, st.m8)
                        if cn == NC - 1:
                            st.mnext = jnp.max(st.m8, axis=0, keepdims=True)
                    else:
                        if cn == NC:
                            st.qt = load_q(u0 + k + 2)
                            st.m8 = None
                        st.m8 = qk_chunk(st.qt, sbuf[k % 2], cn - NC, st.m8)
                    st.hist.append(st.m8)
                    me = st.mc8
                    if st.anchor is not None:
                        me = me + st.anchor * 0.0
                    if len(st.hist) > LAGM:
                        me = me + st.hist[-1 - LAGM] * 0.0
                    sc = sbuf[k % 2][c * 128:(c + 1) * 128, :].reshape(16, 8, 512)
                    p = jnp.exp2(sc - me[None])
                    l8 = st.l8
                    for g in reversed(range(16)):
                        l8 = p[g] if l8 is None else l8 + p[g]
                    st.l8 = l8
                    st.anchor = l8
                    pv = jnp.dot(vt_v[c], p.reshape(128, 512).astype(BF), preferred_element_type=F32)
                    st.acc = pv if st.acc is None else st.acc + pv
                    if c == FIN:
                        finalize(u0 + k - 1, st.pacc, st.pl8 + l8 * 0.0)
                    if c == NC - 1:
                        st.pacc, st.pl8 = st.acc, st.l8
                        st.m = st.mnext
                return run
            for k in range(nu):
                for c in range(NC):
                    tasks.append(mk(k, c))
            return tasks

        def relayout_block(sub, anchor):
            m = lax.shift_right_logical(sub, 8)
            i = lax.shift_right_logical(sub, 2) & 63
            half, par = SUBPAT[0], SUBPAT[1]
            z = pltpu.bitcast(anchor[:, :128] * 0.0, U32)
            msk = z | jnp.uint32(0xFFFF0000 if par else 0xFFFF)
            w = raw_v[m, pl.ds(pl.multiple_of(i * 16, 16), 16), half * 16:(half + 1) * 16, :]
            outs = []
            for t in range(8):
                a = pltpu.bitcast(w[2 * t], U32)
                b = pltpu.bitcast(w[2 * t + 1], U32)
                outs.append(((a >> 16) | (b & msk)) if par else ((a & msk) | (b << 16)))
            tr = jnp.swapaxes(jnp.stack(outs), 0, 1)
            r0 = pl.multiple_of(i * 8, 8)
            for j in range(8):
                wp_v[m, 16 * half + 2 * j + par, pl.ds(r0, 8), :] = tr[j]

        qt0 = load_q(0)
        m8 = None
        for c in range(NC):
            m8 = qk_chunk(qt0, sa_v, c, m8)
        m_init = jnp.max(m8, axis=0, keepdims=True)
        qt1 = load_q(1)
        m8 = None
        for c in range(SKEW):
            m8 = qk_chunk(qt1, sb_v, c, m8)
        carry_a = (m_init, m8, jnp.zeros((DA, 512), F32), jnp.ones((8, 512), F32))

        RPI = 768 // NIT_S
        assert RPI % 4 == 0
        SUBPAT = [0, 0]

        def sa_body(it, carry):
            for m in range(3):
                first = (256 * m) // RPI
                @pl.when(it == first)
                def _():
                    raw_copies[m].wait()
            st = a_state(carry)
            tasks = a_tasks(it * UA, UA, st)
            nt = len(tasks)
            rel_at = {}
            for r_ in range(RPI):
                rel_at.setdefault((r_ * (nt - 2)) // RPI, []).append(r_)
            for n in range(nt):
                tasks[n]()
                if do_rel:
                    for r_ in rel_at.get(n, []):
                        SUBPAT[0], SUBPAT[1] = (r_ >> 1) & 1, r_ & 1
                        relayout_block(it * RPI + r_, st.anchor)
            return a_carry(st)
        with jax.named_scope('P2_attn'):
            carry_a = lax.fori_loop(0, NIT_S, sa_body, carry_a)

        for c in bo_copies:
            c.wait()
        mem_copy.wait()

        r = lax.broadcasted_iota(jnp.int32, (32, 48), 0)
        cc = lax.broadcasted_iota(jnp.int32, (32, 48), 1)
        mask_e = (cc >= 40) | ((cc < 32) & ((cc <= r) | (r >= 24)))
        r = lax.broadcasted_iota(jnp.int32, (48, 80), 0)
        cc = lax.broadcasted_iota(jnp.int32, (48, 80), 1)
        kseg = jnp.where((cc < 32) | ((cc >= 64) & (cc < 72)), 1, 0)
        kpos = jnp.where(cc < 24, cc + 8, jnp.where(cc < 32, -1, jnp.where(cc < 64, cc - 32,
                                                                           jnp.where(cc < 72, cc - 64, -1))))
        qseg = jnp.where(r < 40, 1, 0)
        qpos = jnp.where(r < 24, r + 8, jnp.where(r < 32, 100, jnp.where(r < 40, r - 32, r - 16)))
        mask_o = (kseg == qseg) & (kpos <= qpos)

        def b_step(lhs, even, base, filler):
            mask = mask_e if even else mask_o
            qkv, ps, os_ = {}, {}, {}
            def wmat(m, h):
                return pltpu.bitcast(wp_v[m, h], BF)
            def do_qkv(h):
                q = jnp.dot(lhs, wmat(0, h), preferred_element_type=F32) * SCALE_B
                k = jnp.dot(lhs, wmat(1, h), preferred_element_type=F32).astype(BF)
                v = jnp.dot(lhs, wmat(2, h), preferred_element_type=F32).astype(BF)
                if even:
                    sq_v[h] = jnp.concatenate([q[32:40], q[24:32]], axis=0).astype(BF)
                    skv_v[2 * h] = k
                    skv_v[2 * h + 1] = v
                    q = jnp.concatenate([q[0:24], q[40:48]], axis=0).astype(BF)
                else:
                    q = jnp.concatenate([q.astype(BF), sq_v[h]], axis=0)
                    k = jnp.concatenate([k, skv_v[2 * h]], axis=0)
                    v = jnp.concatenate([v, skv_v[2 * h + 1]], axis=0)
                qkv[h] = (q, k, v)
            def do_s(h):
                q, k, _ = qkv[h]
                s = lax.dot_general(q, k, NT, preferred_element_type=F32)
                s = jnp.where(mask, s, NEG)
                m = jnp.max(s, axis=-1, keepdims=True)
                p = jnp.exp2(s - m)
                l = jnp.sum(p, axis=-1, keepdims=True)
                ps[h] = (p * pl.reciprocal(l, approx=True)).astype(BF)
            def do_pv(h):
                os_[h] = jnp.dot(ps[h], qkv[h][2], preferred_element_type=F32).astype(BF)
            for h in range(HB + L1 + L2):
                if h < HB:
                    do_qkv(h)
                if 0 <= h - L1 < HB:
                    do_s(h - L1)
                if 0 <= h - L1 - L2 < HB:
                    do_pv(h - L1 - L2)
                filler(even, 'head', h)
            ol = jnp.concatenate([os_[h] for h in range(HB)], axis=1)
            ms = []
            for n in range(8):
                y = jnp.dot(ol, bo_v[n], preferred_element_type=F32)
                cols = slice(n * 128, (n + 1) * 128)
                if even:
                    b_v[pl.ds(base, 24), cols] = y[0:24]
                else:
                    b_v[pl.ds(base + 40, 24), cols] = y[0:24]
                    b_v[pl.ds(base + 32, 8), cols] = y[32:40]
                    b_v[pl.ds(base + 24, 8), cols] = y[40:48]
                ms.append(y[24:32].astype(BF))
                filler(even, 'wo', n)
            return jnp.concatenate(ms, axis=1)

        per_step = NC * UF // (2 * PPI)
        crit_e = cfg.get('crit_e', [('head', HB - 1, 1), ('head', HB, 1), ('head', HB + 1, 1), ('wo', 7, 2)])
        crit_o = cfg.get('crit_o', [('head', HB - 1, 1), ('head', HB, 1), ('head', HB + 1, 1), ('wo', 7, 0)])
        ne = cfg.get('ne', per_step)
        slots = {}
        for par, crit, tot in ((True, crit_e, ne), (False, crit_o, 2 * per_step - ne)):
            sl = {(a, b): c for a, b, c in crit}
            rest = tot - sum(sl.values())
            for t in range(rest):
                key = ('head', (t * (HB - 2)) // rest + 1)
                sl[key] = sl.get(key, 0) + 1
            for k_, v_ in sl.items():
                slots[(par,) + k_] = v_
        assert sum(slots.values()) == 2 * per_step

        def fused_body(t, carry):
            mem = carry[0]
            st = a_state(carry[1:])
            tasks = a_tasks(NU_S + t * UF, UF, st)
            it = iter(tasks)
            def filler(even, kind, idx):
                for _ in range(slots.get((even, kind, idx), 0)):
                    next(it)()
            for pp in range(PPI):
                base = pl.multiple_of((t * PPI + pp) * 64, 64)
                mem = b_step(jnp.concatenate([x_v[pl.ds(base, 40), :], mem], axis=0), True, base, filler)
                mem = b_step(jnp.concatenate([x_v[pl.ds(base + 40, 24), :], mem], axis=0), False, base, filler)
            return (mem,) + a_carry(st)
        with jax.named_scope('P3_fused'):
            carry = lax.fori_loop(0, NIT_F, fused_body, (mem0_v[...],) + carry_a)
        finalize(NUNITS - 1, carry[3], carry[4])

        wo_copy.wait()
        gw_copy.wait()
        gw = gw_v[...].astype(F32)

        def out_copy(i, slot):
            return pltpu.make_async_copy(ob_v.at[slot], out_hbm.at[pl.ds(i * OB, OB)], osem.at[slot])

        def epi_body(i, carry):
            slot = i & 1
            r0 = pl.multiple_of(i * OB, OB)
            @pl.when(i >= 2)
            def _():
                out_copy(i - 2, slot).wait()
            ol = jnp.concatenate([o_v[g, pl.ds(r0, OB), :] for g in range(8)], axis=1)
            a = jnp.dot(ol, wo_v[...], preferred_element_type=F32)
            xg = None
            for g in range(8):
                t = x_v[pl.ds(r0, OB), g * 128:(g + 1) * 128].astype(F32) * gw[g:g + 1, :]
                xg = t if xg is None else xg + t
            logit = jnp.sum(xg, axis=-1, keepdims=True)
            g_ = jax.nn.sigmoid(logit)
            bb = b_v[pl.ds(r0, OB), :]
            ob_v[slot] = (g_ * a + (1.0 - g_) * bb).astype(BF)
            out_copy(i, slot).start()
            return carry
        with jax.named_scope('P4_epi'):
            lax.fori_loop(0, S // OB, epi_body, 0)
        out_copy(S // OB - 2, 0).wait()
        out_copy(S // OB - 1, 1).wait()

    def fn(A_x, A_wq, A_wk, A_wv, A_wo, B_x, B_mem0, B_Wq, B_Wk, B_Wv, B_Wo, B_seg_len, gate_w):
        any_spec = pl.BlockSpec(memory_space=pl.ANY)
        out = pl.pallas_call(
            kernel,
            out_shape=jax.ShapeDtypeStruct((S, D), BF),
            in_specs=[any_spec] * 11,
            out_specs=any_spec,
            scratch_shapes=[
                pltpu.VMEM((S, D), BF),
                pltpu.VMEM((4, D, 256), BF),
                pltpu.VMEM((D, D), BF),
                pltpu.VMEM((2 * DA, D), BF),
                pltpu.VMEM((8, D), BF),
                pltpu.VMEM((8, 128), BF),
                pltpu.VMEM((3, D, HB, DB), BF),
                pltpu.VMEM((3, HB, D // 2, DB), U32),
                pltpu.VMEM((8, HB * DB, 128), BF),
                pltpu.VMEM((NQT, D, 128), BF),
                pltpu.VMEM((S, DA), BF),
                pltpu.VMEM((NC, DA, 128), BF),
                pltpu.VMEM((S, 512), F32),
                pltpu.VMEM((S, 512), F32),
                pltpu.VMEM((8, S, 128), BF),
                pltpu.VMEM((S, D), F32),
                pltpu.VMEM((HB, 16, DB), BF),
                pltpu.VMEM((2 * HB, 48, DB), BF),
                pltpu.VMEM((2, OB, D), BF),
                pltpu.SemaphoreType.DMA((NXB,)),
                pltpu.SemaphoreType.DMA((4,)),
                pltpu.SemaphoreType.DMA((8,)),
                pltpu.SemaphoreType.DMA((8,)),
                pltpu.SemaphoreType.DMA((2,)),
            ],
            compiler_params=pltpu.CompilerParams(vmem_limit_bytes=120 * 1024 * 1024),
        )(A_x.reshape(S, D), A_wq, A_wk.T, A_wv.T, A_wo, B_mem0.reshape(8, D), B_Wq, B_Wk, B_Wv,
          B_Wo.reshape(HB * DB, D), gate_w.reshape(8, 128))
        return out.reshape(1, S, D)
    return jax.jit(fn)


_FN = build({"SKEW": 3, "UA": 8})


@jax.jit
def pallas_gated_mix__grouped_kv_mqa__memory_aug_recurrent_mem_tr__prompt_kernel(
    A_x: jax.Array,
    A_wq: jax.Array,
    A_wk: jax.Array,
    A_wv: jax.Array,
    A_wo: jax.Array,
    B_x: jax.Array,
    B_mem0: jax.Array,
    B_Wq: jax.Array,
    B_Wk: jax.Array,
    B_Wv: jax.Array,
    B_Wo: jax.Array,
    B_seg_len: jax.Array,
    gate_w: jax.Array,
):
    return _FN(A_x, A_wq, A_wk, A_wv, A_wo, B_x, B_mem0, B_Wq, B_Wk, B_Wv, B_Wo, B_seg_len, gate_w)
```

```python
import functools
import jax
import jax.numpy as jnp
import numpy as np
from jax import lax
import jax.experimental.pallas as pl
import jax.experimental.pallas.tpu as pltpu

BF = jnp.bfloat16
F32 = jnp.float32
U32 = jnp.uint32

S = 2048
D = 1024
HA, DA = 32, 32
HB, DB = 32, 128
LOG2E = 1.4426950408889634
SCALE_A = float(np.asarray(DA ** -0.5, dtype=BF)) * LOG2E
SCALE_B = float(np.asarray(DB ** -0.5, dtype=BF)) * LOG2E
NEG = -1e30

XB = 256
NXB = S // XB
NQT = S // 128
NUNITS = NQT * (HA // 4)
NC = S // 128
OB = 256
NT = (((1,), (1,)), ((), ()))


def build(cfg):
    do_a = cfg.get('a', True); do_b = cfg.get('b', True); do_rel = cfg.get('rel', True)
    UA = cfg.get('UA', 4)
    PPI = cfg.get('PPI', 1)
    UF = cfg.get('UF', 2)
    SKEW = cfg.get('SKEW', 3)
    AG = cfg.get('AG', 0)
    LAGM = cfg.get('LAGM', 2)
    FG = cfg.get('FG', 0)
    EXT = cfg.get('EXT', 0)
    BANC = cfg.get('BANC', 1)
    FIN = cfg.get('FIN', 0)
    NPAIR = S // 64
    NIT_F = NPAIR // PPI
    NU_F = UF * NIT_F
    NU_S = NUNITS - NU_F
    NIT_S = NU_S // UA
    NPRE = cfg.get('NPRE', 4)
    TPI = cfg.get('TPI', UA // 4)
    FOLD = cfg.get('FOLD', 1)
    QROWS = cfg.get('QROWS', 256)
    NIT_B = (NQT - NPRE) // TPI if FOLD else cfg.get('NIT_B', 16)
    NIT_A = NIT_S - NIT_B
    WQG = cfg.get('WQG', 4)
    XSTART = cfg.get('XSTART', -1)
    QPOS = cfg.get('QPOS', [14, 15])
    QAT = cfg.get('QAT', [-1, -1] + [k * NC + p for k in range(UA - 1) for p in QPOS])
    RSKIP = cfg.get('RSKIP', [])
    L1 = cfg.get('L1', 1)
    L2E, L2O = cfg.get('L2E', 3), cfg.get('L2O', 3)
    assert UA % 2 == 0 and NU_S % UA == 0 and 768 % NIT_B == 0 and (len(QAT) == 8 * TPI or not FOLD)

    def kernel(x_hbm, wq_hbm, wkt_hbm, wvt_hbm, wo_hbm, mem0_hbm, bq_hbm, bk_hbm, bv_hbm, bo_hbm, gw_hbm,
               out_hbm,
               x_v, wq_v, wo_v, wkv_v, mem0_v, gw_v, raw_v, wp_v, bo_v, qt_v, k_v, vt_v, sa_v, sb_v, sc_v, o_v, b_v,
               sq_v, skv_v, ob_v, g_v,
               xsem, wqsem, wsem, bosem, wosem, osem):
        sbuf = (sa_v, sb_v, sc_v)

        def x_copy(i):
            return pltpu.make_async_copy(x_hbm.at[pl.ds(i * XB, XB)], x_v.at[pl.ds(i * XB, XB)], xsem.at[i])
        wq_copies = [pltpu.make_async_copy(wq_hbm.at[:, pl.ds(n * 128, 128)], wq_v.at[n], wqsem.at[n])
                     for n in range(8)]
        wo_copies = [pltpu.make_async_copy(wo_hbm.at[:, pl.ds(n * 128, 128)], wo_v.at[n], wosem.at[n])
                     for n in range(8)]
        raw_copies = [pltpu.make_async_copy(src, raw_v.at[m], wsem.at[1 + m])
                      for m, src in enumerate((bq_hbm, bk_hbm, bv_hbm))]
        wk_copy = pltpu.make_async_copy(wkt_hbm, wkv_v.at[pl.ds(0, DA)], wsem.at[4])
        wv_copy = pltpu.make_async_copy(wvt_hbm, wkv_v.at[pl.ds(DA, DA)], wsem.at[5])
        mem_copy = pltpu.make_async_copy(mem0_hbm, mem0_v, wsem.at[6])
        gw_copy = pltpu.make_async_copy(gw_hbm, gw_v, wsem.at[7])
        bo_copies = [pltpu.make_async_copy(bo_hbm.at[:, pl.ds(n * 128, 128)], bo_v.at[n], bosem.at[n])
                     for n in range(8)]

        wk_copy.start()
        wv_copy.start()
        gw_copy.start()
        x_copy(0).start()
        wk_copy.wait()
        wv_copy.wait()
        gw_copy.wait()
        for c in wq_copies:
            c.start()

        def kv_proj(rb):
            xb = x_v[rb * XB:(rb + 1) * XB, :]
            kvt = lax.dot_general(wkv_v[...], xb, NT, preferred_element_type=F32)
            k_v[rb * XB:(rb + 1) * XB, :] = kvt[:DA].T.astype(BF)
            for t in range(XB // 128):
                vt_v[rb * (XB // 128) + t] = kvt[DA:2 * DA, t * 128:(t + 1) * 128].astype(BF)

        def q_piece(tile, n, rows=128):
            r0 = tile * 128 if isinstance(tile, int) else pl.multiple_of(tile * 128, 128)
            q = jnp.dot(x_v[pl.ds(r0, rows), :], wq_v[n], preferred_element_type=F32) * SCALE_A
            for t in range(rows // 128):
                qt_v[tile + t, n * 128:(n + 1) * 128, :] = q[t * 128:(t + 1) * 128].T.astype(BF)
            return q[FG * 8:FG * 8 + 8]

        with jax.named_scope('P1_proj'):
            x_copy(0).wait()
            if XSTART < 0:
                for i in range(1, NXB):
                    x_copy(i).start()
            kv_proj(0)
            for n in range(8):
                if n % WQG == 0:
                    for c in wq_copies[n:n + WQG]:
                        c.wait()
                if n == XSTART:
                    for i in range(1, NXB):
                        x_copy(i).start()
                q_piece(0, n, XB)
            for rb in range(1, NPRE * 128 // XB):
                x_copy(rb).wait()
                kv_proj(rb)
                for n in range(8):
                    q_piece(rb * (XB // 128), n, XB)
            for rb in range(NPRE * 128 // XB, NXB):
                x_copy(rb).wait()
            for c in raw_copies + bo_copies + wo_copies + [mem_copy]:
                c.start()
            for rb in range(NPRE * 128 // XB, NXB):
                kv_proj(rb)
            if not FOLD:
                for tile in range(NPRE, NQT, QROWS // 128):
                    for n in range(8):
                        q_piece(tile, n, QROWS)

        def load_q(u):
            u = jnp.minimum(u, NUNITS - 1)
            qi = lax.shift_right_logical(u, 3)
            base = pl.multiple_of((u & 7) * 128, 128)
            return jnp.concatenate(
                [qt_v[qi, pl.ds(base + 32 * j, 32), :] for j in range(4)], axis=1)

        first = [None]
        def qk_chunk(qt, s_ref, c, m8):
            sn = jnp.dot(k_v[c * 128:(c + 1) * 128, :], qt, preferred_element_type=F32)
            s_ref[c * 128:(c + 1) * 128, :] = sn
            for g in range(16):
                t = sn[g * 8:(g + 1) * 8]
                m8 = t if m8 is None else jnp.maximum(m8, t)
            first[0] = sn[FG * 8:FG * 8 + 8, 0:128]
            return m8

        def finalize(u, acc, l8):
            u = jnp.maximum(u, 0)
            l = jnp.sum(l8, axis=0, keepdims=True)
            inv = pl.reciprocal(l, approx=True)
            o = acc * inv
            o4 = jnp.concatenate([o[:, j * 128:(j + 1) * 128] for j in range(4)], axis=0)
            row = pl.multiple_of(lax.shift_right_logical(u, 3) * 128, 128)
            ot = o4.T
            o_v[u & 7, pl.ds(row, 128), :] = ot.astype(BF)
            return ot[120:128]

        class AState:
            pass

        def a_state(carry):
            st = AState()
            st.m, st.m8, st.pacc, st.pl8 = carry
            st.anchor = None
            st.hist = []
            st.ext = None
            return st

        def a_carry(st):
            return st.m, st.m8, st.pacc, st.pl8

        def a_tasks(u0, nu, st):
            tasks = []
            if cfg.get('PRELOAD', 1):
                qts = [load_q(u0 + 1 + j) for j in range(nu + 1)]
                getq = lambda j: qts[j]
            else:
                getq = lambda j: load_q(u0 + 1 + j)
            def mk(k, c):
                def run():
                    if c == 0:
                        st.mc8 = jnp.broadcast_to(st.m, (8, 512))
                        st.l8 = None
                        st.acc = None
                    ext = st.ext
                    cn = c + SKEW
                    if cn < NC:
                        if c == 0 and k == 0:
                            st.qt = getq(k)
                        st.m8 = qk_chunk(st.qt, sbuf[(k + 1) % 2], cn, st.m8)
                        if cn == NC - 1:
                            st.mnext = jnp.max(st.m8, axis=0, keepdims=True)
                    else:
                        if cn == NC:
                            st.qt = getq(k + 1)
                            st.m8 = None
                        st.m8 = qk_chunk(st.qt, sbuf[k % 2], cn - NC, st.m8)
                    st.hist.append(st.m8)
                    me = st.mc8
                    if st.anchor is not None:
                        me = me + st.anchor * 0.0
                    if len(st.hist) > LAGM:
                        me = me + st.hist[-1 - LAGM] * 0.0
                    if ext is not None and EXT:
                        z = ext * 0.0
                        me = me + jnp.concatenate([z, z, z, z], axis=1)
                    st.ext = first[0]
                    sc = sbuf[k % 2][c * 128:(c + 1) * 128, :].reshape(16, 8, 512)
                    p = jnp.exp2(sc - me[None])
                    l8 = st.l8
                    for g in reversed(range(16)):
                        l8 = p[g] if l8 is None else l8 + p[g]
                        if g == AG:
                            st.anchor = l8
                    st.l8 = l8
                    pv = jnp.dot(vt_v[c], p.reshape(128, 512).astype(BF), preferred_element_type=F32)
                    st.acc = pv if st.acc is None else st.acc + pv
                    if c == FIN:
                        finalize(u0 + k - 1, st.pacc, st.pl8 + l8 * 0.0)
                    if c == NC - 1:
                        st.pacc, st.pl8 = st.acc, st.l8
                        st.m = st.mnext
                return run
            for k in range(nu):
                for c in range(NC):
                    tasks.append(mk(k, c))
            return tasks

        def relayout_block(sub, anchor):
            m = lax.shift_right_logical(sub, 8)
            i = lax.shift_right_logical(sub, 2) & 63
            half, par = SUBPAT[0], SUBPAT[1]
            z = pltpu.bitcast(anchor[:, :128] * 0.0, U32)
            msk = z | jnp.uint32(0xFFFF0000 if par else 0xFFFF)
            w = raw_v[m, pl.ds(pl.multiple_of(i * 16, 16), 16), half * 16:(half + 1) * 16, :]
            outs = []
            for t in range(8):
                a = pltpu.bitcast(w[2 * t], U32)
                b = pltpu.bitcast(w[2 * t + 1], U32)
                outs.append(((a >> 16) | (b & msk)) if par else ((a & msk) | (b << 16)))
            tr = jnp.swapaxes(jnp.stack(outs), 0, 1)
            r0 = pl.multiple_of(i * 8, 8)
            for j in range(8):
                wp_v[m, 16 * half + 2 * j + par, pl.ds(r0, 8), :] = tr[j]

        def gate_block(r0, rows, anchor):
            gw = gw_v[...].astype(F32)
            xg = jnp.concatenate([anchor[:, :128] * 0.0] * (rows // 8), axis=0)
            for g in range(8):
                xg = xg + x_v[pl.ds(r0, rows), g * 128:(g + 1) * 128].astype(F32) * gw[g:g + 1, :]
            gt = jax.nn.sigmoid(jnp.sum(xg, axis=-1, keepdims=True))
            gt = jnp.broadcast_to(gt, (rows, 128))
            g_v[pl.ds(r0, rows), :] = gt
            return jnp.sum(gt.reshape(rows // 8, 8, 128), axis=0)

        qt0 = load_q(0)
        m8 = None
        for c in range(NC):
            m8 = qk_chunk(qt0, sa_v, c, m8)
        m_init = jnp.max(m8, axis=0, keepdims=True)
        qt1 = load_q(1)
        m8 = None
        for c in range(SKEW):
            m8 = qk_chunk(qt1, sb_v, c, m8)
        carry_a = (m_init, m8, jnp.zeros((DA, 512), F32), jnp.ones((8, 512), F32))

        RPI = 768 // NIT_B
        assert RPI % 4 == 0
        SUBPAT = [0, 0]

        def sa_body(it, carry):
            st = a_state(carry)
            for task in a_tasks(it * UA, UA, st):
                task()
            return a_carry(st)

        def sb_body(it, carry):
            for m in range(3):
                first = (256 * m) // RPI
                @pl.when(it == first)
                def _():
                    raw_copies[m].wait()
            st = a_state(carry)
            tasks = a_tasks((NIT_A + it) * UA, UA, st)
            nt = len(tasks)
            rel_ok = [n for n in range(nt) if (n % NC) not in RSKIP]
            rel_at = {}
            for r_ in range(RPI):
                rel_at.setdefault(rel_ok[(r_ * len(rel_ok)) // RPI], []).append(r_)
            qn = 0
            for _ in range(QAT.count(-1) if FOLD else 0):
                q_piece(NPRE + it * TPI + qn // 8, qn % 8)
                qn += 1
            for n in range(nt):
                tasks[n]()
                if do_rel:
                    for r_ in rel_at.get(n, []):
                        SUBPAT[0], SUBPAT[1] = (r_ >> 1) & 1, r_ & 1
                        relayout_block(it * RPI + r_, st.anchor)
                for _ in range(QAT.count(n) if FOLD else 0):
                    st.ext = q_piece(NPRE + it * TPI + qn // 8, qn % 8)
                    qn += 1
            return a_carry(st)
        if NIT_A:
            with jax.named_scope('P2a_attn'):
                carry_a = lax.fori_loop(0, NIT_A, sa_body, carry_a)
        with jax.named_scope('P2b_attn'):
            carry_a = lax.fori_loop(0, NIT_B, sb_body, carry_a)

        for c in bo_copies + wo_copies:
            c.wait()
        mem_copy.wait()

        def out_piece(r0, rows, n, slot, off):
            ol = jnp.concatenate([o_v[g, pl.ds(r0, rows), :] for g in range(8)], axis=1)
            a = jnp.dot(ol, wo_v[n], preferred_element_type=F32)
            g_ = g_v[pl.ds(r0, rows), :]
            bb = b_v[pl.ds(r0, rows), n * 128:(n + 1) * 128]
            res = g_ * a + (1.0 - g_) * bb
            ob_v[slot, off:off + rows, n * 128:(n + 1) * 128] = res.astype(BF)
            return res

        def out_copy(i, slot):
            return pltpu.make_async_copy(ob_v.at[slot], out_hbm.at[pl.ds(i * OB, OB)], osem.at[slot])

        r = lax.broadcasted_iota(jnp.int32, (32, 48), 0)
        cc = lax.broadcasted_iota(jnp.int32, (32, 48), 1)
        mask_e = (cc >= 40) | ((cc < 32) & ((cc <= r) | (r >= 24)))
        r = lax.broadcasted_iota(jnp.int32, (48, 80), 0)
        cc = lax.broadcasted_iota(jnp.int32, (48, 80), 1)
        kseg = jnp.where((cc < 32) | ((cc >= 64) & (cc < 72)), 1, 0)
        kpos = jnp.where(cc < 24, cc + 8, jnp.where(cc < 32, -1, jnp.where(cc < 64, cc - 32,
                                                                           jnp.where(cc < 72, cc - 64, -1))))
        qseg = jnp.where(r < 40, 1, 0)
        qpos = jnp.where(r < 24, r + 8, jnp.where(r < 32, 100, jnp.where(r < 40, r - 32, r - 16)))
        mask_o = (kseg == qseg) & (kpos <= qpos)

        def b_step(lhs, even, base, hook, zget):
            mask = mask_e if even else mask_o
            L2 = L2E if even else L2O
            qkv, ps, os_ = {}, {}, {}
            def wmat(m, h):
                return pltpu.bitcast(wp_v[m, h], BF)
            def do_qkv(h):
                q = jnp.dot(lhs, wmat(0, h), preferred_element_type=F32) * SCALE_B
                hook(even, 'dot', 3 * h)
                k = jnp.dot(lhs, wmat(1, h), preferred_element_type=F32).astype(BF)
                hook(even, 'dot', 3 * h + 1)
                v = jnp.dot(lhs, wmat(2, h), preferred_element_type=F32).astype(BF)
                hook(even, 'dot', 3 * h + 2)
                z = zget()
                q0 = q[0:8] if z is None else q[0:8] + z
                if even:
                    sq_v[h] = jnp.concatenate([q[32:40], q[24:32]], axis=0).astype(BF)
                    skv_v[2 * h] = k
                    skv_v[2 * h + 1] = v
                    q = jnp.concatenate([q0, q[8:24], q[40:48]], axis=0).astype(BF)
                else:
                    q = jnp.concatenate([jnp.concatenate([q0, q[8:32]], axis=0).astype(BF), sq_v[h]], axis=0)
                    k = jnp.concatenate([k, skv_v[2 * h]], axis=0)
                    v = jnp.concatenate([v, skv_v[2 * h + 1]], axis=0)
                qkv[h] = (q, k, v)
            def do_s(h):
                q, k, _ = qkv[h]
                s = lax.dot_general(q, k, NT, preferred_element_type=F32)
                s = jnp.where(mask, s, NEG)
                m = jnp.max(s, axis=-1, keepdims=True)
                p = jnp.exp2(s - m)
                l = jnp.sum(p, axis=-1, keepdims=True)
                ps[h] = (p * pl.reciprocal(l, approx=True)).astype(BF)
            def do_pv(h):
                o = jnp.dot(ps[h], qkv[h][2], preferred_element_type=F32)
                if h == HB - 1:
                    z = zget()
                    if z is not None:
                        o = jnp.concatenate([o[0:8] + z, o[8:]], axis=0)
                os_[h] = o.astype(BF)
            for h in range(HB + L1 + L2):
                if h < HB:
                    do_qkv(h)
                if 0 <= h - L1 < HB:
                    do_s(h - L1)
                if 0 <= h - L1 - L2 < HB:
                    do_pv(h - L1 - L2)
                hook(even, 'head', h)
            ms = []
            nq = WOQ if even else 1
            hq = HB // nq
            ols = [jnp.concatenate([os_[h] for h in range(j * hq, (j + 1) * hq)], axis=1) for j in range(nq)]
            for n in range(8):
                y = None
                for j in range(nq):
                    t = jnp.dot(ols[j], bo_v[n, j * hq * DB:(j + 1) * hq * DB, :], preferred_element_type=F32)
                    y = t if y is None else y + t
                    hook(even, 'woq', n * nq + j)
                cols = slice(n * 128, (n + 1) * 128)
                if even:
                    b_v[pl.ds(base, 24), cols] = y[0:24]
                else:
                    b_v[pl.ds(base + 40, 24), cols] = y[0:24]
                    b_v[pl.ds(base + 32, 8), cols] = y[32:40]
                    b_v[pl.ds(base + 24, 8), cols] = y[40:48]
                z = zget() if n >= 2 else None
                ms.append((y[24:32] if z is None else y[24:32] + z).astype(BF))
            return jnp.concatenate(ms, axis=1)

        WOQ = cfg.get('WOQ', 4)
        MK = cfg.get('MK', 32)
        MPC = 128 // MK
        ZLAG = cfg.get('ZLAG', 4)
        OLAG = cfg.get('OLAG', 1)
        GAT = cfg.get('GAT', [5, 9, 20, 24])
        FLAG = cfg.get('FLAG', 2)
        TRE = cfg.get('TRE', [4, 4, 4, 4])
        TRO = cfg.get('TRO', [4, 4, 4, 4])
        ENDE = cfg.get('ENDE', 5)
        WOE = cfg.get('WOE', 1)
        pv_slots, qk_slots = {}, {}
        npv = NC * UF
        for i in range(npv):
            key = (True, 'dot', 3 * ((i * HB) // npv) + 2 - ((i * HB) % npv != 0 and UF > 2 and (i % 3 == 1)))
            pv_slots[key] = pv_slots.get(key, 0) + 1
        sc = 32 // MK if MK <= 32 else 1
        def addq(key, cnt):
            qk_slots[key] = qk_slots.get(key, 0) + cnt
        for j, cnt in enumerate(TRE):
            addq((True, 'head', HB - 1 + j), cnt * 32 // MK)
        for j, cnt in enumerate(TRO):
            addq((False, 'head', HB - 1 + j), cnt * 32 // MK)
        for j in range(8 * WOQ - 1):
            if (j % cfg.get('WOSTEP', 2)) == 0:
                addq((True, 'woq', j), WOE)
        addq((True, 'woq', 8 * WOQ - 1), ENDE * 32 // MK)
        rest = NC * UF * MPC - sum(qk_slots.values())
        NDOT = 3 * HB - 3
        for i in range(rest):
            addq((False, 'dot', (i * NDOT) // rest), 1)
        assert sum(qk_slots.values()) == NC * UF * MPC and rest >= 0

        op_slots = {}
        for key in cfg.get('OPS', [(1, 'head', 31), (1, 'head', 32), (1, 'head', 33), (1, 'woq', 15), (1, 'woq', 31),
                                   (0, 'dot', 11), (0, 'dot', 23), (0, 'dot', 35), (0, 'dot', 47), (0, 'dot', 59),
                                   (0, 'dot', 71), (0, 'dot', 83), (0, 'head', 31), (0, 'head', 32), (0, 'head', 33),
                                   (0, 'head', 34)]):
            key = (bool(key[0]), key[1], key[2])
            op_slots[key] = op_slots.get(key, 0) + 1
        assert sum(op_slots.values()) == 16

        def fused_body(t, carry, last=False):
            mem = carry[0]
            u0 = NU_S + t * UF
            st = AState()
            st.pv, st.qk, st.l8, st.acc, st.prev = 0, 0, None, None, None
            st.m8, st.hist, st.used, st.mn, st.fin = None, [], 0, [], []

            def pv_task():
                k, c = divmod(st.pv, NC)
                st.pv += 1
                if c == 0:
                    st.mc8 = jnp.broadcast_to(carry[1 + k], (8, 512))
                    st.l8, st.acc = None, None
                me = st.mc8 if st.prev is None else st.mc8 + st.prev * 0.0
                p = jnp.exp2(sbuf[k][c * 128:(c + 1) * 128, :].reshape(16, 8, 512) - me[None])
                l8 = st.l8
                for g in reversed(range(16)):
                    l8 = p[g] if l8 is None else l8 + p[g]
                st.l8 = st.prev = l8
                pv = jnp.dot(vt_v[c], p.reshape(128, 512).astype(BF), preferred_element_type=F32)
                st.acc = pv if st.acc is None else st.acc + pv
                if c == NC - 1:
                    st.fin.append((FLAG, finalize(u0 + k, st.acc, st.l8)))

            def qk_piece():
                k, i = divmod(st.qk, NC * MPC)
                st.qk += 1
                assert st.pv > k * NC + (i * MK) // 128
                if i == 0:
                    st.qt = load_q(u0 + UF + k)
                    st.m8 = None
                sn = jnp.dot(k_v[i * MK:(i + 1) * MK, :], st.qt, preferred_element_type=F32)
                sbuf[k][i * MK:(i + 1) * MK, :] = sn
                m8 = st.m8
                for g in range(MK // 8):
                    tt = sn[g * 8:(g + 1) * 8]
                    m8 = tt if m8 is None else jnp.maximum(m8, tt)
                st.m8 = m8
                st.hist.append(m8)
                if i == NC * MPC - 1:
                    st.mn.append(jnp.max(m8, axis=0, keepdims=True))

            def hook(even, kind, idx):
                if even and kind == 'head' and idx in GAT:
                    gi = GAT.index(idx)
                    gr = 64 // len(GAT)
                    st.fin.append((FLAG, gate_block(base + gi * gr, gr, st.prev)))
                for _ in range(pv_slots.get((even, kind, idx), 0)):
                    pv_task()
                if not last:
                    for _ in range(qk_slots.get((even, kind, idx), 0)):
                        qk_piece()
                else:
                    for _ in range(op_slots.get((even, kind, idx), 0)):
                        half, n = divmod(st.op, 8)
                        st.op += 1
                        res = out_piece(half * 128, 128, n, 0, half * 128)
                        st.hist.append(jnp.sum(res.reshape(16, 8, 128), axis=0))

            def zget():
                z = None
                if st.fin and st.fin[0][0] <= 0:
                    z = st.fin.pop(0)[1]
                st.fin = [(a_ - 1, b_) for a_, b_ in st.fin]
                n = len(st.hist) - (OLAG if last else ZLAG)
                if n > st.used:
                    vals = st.hist[st.used:n] if last else st.hist[n - 1:n]
                    st.used = n
                    for m8 in vals:
                        if not last:
                            m8 = (m8[:, 0:128] + m8[:, 128:256]) + (m8[:, 256:384] + m8[:, 384:512])
                        z = m8 if z is None else z + m8
                return None if z is None else z * 0.0

            if last:
                st.op = 0
            base = t * 64 if last else pl.multiple_of(t * 64, 64)
            mem = b_step(jnp.concatenate([x_v[pl.ds(base, 40), :], mem], axis=0), True, base, hook, zget)
            mem = b_step(jnp.concatenate([x_v[pl.ds(base + 40, 24), :], mem], axis=0), False, base, hook, zget)
            return (mem,) + tuple(st.mn)

        finalize(NU_S - 1, carry_a[2], carry_a[3])
        ms0 = [carry_a[0]]
        for k in range(1, UF):
            qtb = load_q(NU_S + k)
            m8 = carry_a[1] if k == 1 else None
            for c in range(SKEW if k == 1 else 0, NC):
                m8 = qk_chunk(qtb, sbuf[k], c, m8)
            ms0.append(jnp.max(m8, axis=0, keepdims=True))
        with jax.named_scope('P3_fused'):
            carry = lax.fori_loop(0, NIT_F - 1, fused_body, (mem0_v[...],) + tuple(ms0))
        with jax.named_scope('P3_last'):
            fused_body(NIT_F - 1, carry, last=True)
        out_copy(0, 0).start()

        def epi_body(i, carry):
            slot = i & 1
            r0 = pl.multiple_of(i * OB, OB)
            @pl.when(i >= 2)
            def _():
                out_copy(i - 2, slot).wait()
            for n in range(8):
                out_piece(r0, OB, n, slot, 0)
            out_copy(i, slot).start()
            return carry
        with jax.named_scope('P4_epi'):
            lax.fori_loop(1, S // OB, epi_body, 0)
        out_copy(S // OB - 2, 0).wait()
        out_copy(S // OB - 1, 1).wait()

    def fn(A_x, A_wq, A_wk, A_wv, A_wo, B_x, B_mem0, B_Wq, B_Wk, B_Wv, B_Wo, B_seg_len, gate_w):
        any_spec = pl.BlockSpec(memory_space=pl.ANY)
        out = pl.pallas_call(
            kernel,
            out_shape=jax.ShapeDtypeStruct((S, D), BF),
            in_specs=[any_spec] * 11,
            out_specs=any_spec,
            scratch_shapes=[
                pltpu.VMEM((S, D), BF),
                pltpu.VMEM((8, D, 128), BF),
                pltpu.VMEM((8, D, 128), BF),
                pltpu.VMEM((2 * DA, D), BF),
                pltpu.VMEM((8, D), BF),
                pltpu.VMEM((8, 128), BF),
                pltpu.VMEM((3, D, HB, DB), BF),
                pltpu.VMEM((3, HB, D // 2, DB), U32),
                pltpu.VMEM((8, HB * DB, 128), BF),
                pltpu.VMEM((NQT, D, 128), BF),
                pltpu.VMEM((S, DA), BF),
                pltpu.VMEM((NC, DA, 128), BF),
                pltpu.VMEM((S, 512), F32),
                pltpu.VMEM((S, 512), F32),
                pltpu.VMEM((S if UF > 2 else 8, 512), F32),
                pltpu.VMEM((8, S, 128), BF),
                pltpu.VMEM((S, D), F32),
                pltpu.VMEM((HB, 16, DB), BF),
                pltpu.VMEM((2 * HB, 48, DB), BF),
                pltpu.VMEM((2, OB, D), BF),
                pltpu.VMEM((S, 128), F32),
                pltpu.SemaphoreType.DMA((NXB,)),
                pltpu.SemaphoreType.DMA((8,)),
                pltpu.SemaphoreType.DMA((8,)),
                pltpu.SemaphoreType.DMA((8,)),
                pltpu.SemaphoreType.DMA((8,)),
                pltpu.SemaphoreType.DMA((2,)),
            ],
            compiler_params=pltpu.CompilerParams(vmem_limit_bytes=120 * 1024 * 1024),
        )(A_x.reshape(S, D), A_wq, A_wk.T, A_wv.T, A_wo, B_mem0.reshape(8, D), B_Wq, B_Wk, B_Wv,
          B_Wo.reshape(HB * DB, D), gate_w.reshape(8, 128))
        return out.reshape(1, S, D)
    return jax.jit(fn)


_FN = build({"AG": 8, "SKEW": 2})


@jax.jit
def pallas_gated_mix__grouped_kv_mqa__memory_aug_recurrent_mem_tr__prompt_kernel(
    A_x: jax.Array,
    A_wq: jax.Array,
    A_wk: jax.Array,
    A_wv: jax.Array,
    A_wo: jax.Array,
    B_x: jax.Array,
    B_mem0: jax.Array,
    B_Wq: jax.Array,
    B_Wk: jax.Array,
    B_Wv: jax.Array,
    B_Wo: jax.Array,
    B_seg_len: jax.Array,
    gate_w: jax.Array,
):
    return _FN(A_x, A_wq, A_wk, A_wv, A_wo, B_x, B_mem0, B_Wq, B_Wk, B_Wv, B_Wo, B_seg_len, gate_w)
```

```python
import jax
import jax.numpy as jnp
import numpy as np
from jax import lax
import jax.experimental.pallas as pl
import jax.experimental.pallas.tpu as pltpu

BF = jnp.bfloat16
F32 = jnp.float32
U32 = jnp.uint32

S = 2048
D = 1024
HA, DA = 32, 32
HB, DB = 32, 128
LOG2E = 1.4426950408889634
SCALE_A = float(np.asarray(DA ** -0.5, dtype=BF)) * LOG2E
SCALE_B = float(np.asarray(DB ** -0.5, dtype=BF)) * LOG2E
MASKED = float(np.asarray(-1e9, dtype=BF)) * LOG2E

XB = 256
NXB = S // XB
NQT = S // 128
NUNITS = NQT * (HA // 4)
NC = S // 128
OB = 256
NPAIR = S // 64
NT = (((1,), (1,)), ((), ()))


class _State:
    pass


def build(cfg):
    UA = cfg.get('UA', 4)
    QPI = 2 * UA
    UF = 2
    NU_S = NUNITS - UF * NPAIR
    NPG = 2
    NIT_B = (8 - NPG) * NQT // QPI
    NIT_A = NU_S // UA - NIT_B
    RPI = 768 // NIT_B
    SKEW = cfg.get('SKEW', 2)
    AG = cfg.get('AG', 8)
    LAGM = cfg.get('LAGM', 2)
    FIN = cfg.get('FIN', 0)
    QAT = cfg.get('QAT', [-1, -1] + [NC * k + p for k in range(UA - 1) for p in (14, 15)])
    xw = cfg.get('XW', [1, 3, 5, 8])
    XWAIT = dict(zip(xw[:-1], xw[1:]))
    L1 = cfg.get('L1', 1)
    L2E, L2O = cfg.get('L2E', 3), cfg.get('L2O', 3)
    WOQ = cfg.get('WOQ', 4)
    MK = 32
    MPC = 128 // MK
    ZLAG, OLAG, FLAG = cfg.get('ZLAG', 4), cfg.get('OLAG', 1), cfg.get('FLAG', 2)
    GAT = cfg.get('GAT', [5, 9, 20, 24])
    PVD = cfg.get('PVD', 2)

    pv_slots = {(True, 'dot', 3 * h + PVD): 1 for h in range(NC * UF)}
    qk_slots = {}
    def addq(key, cnt):
        qk_slots[key] = qk_slots.get(key, 0) + cnt
    for j, cnt in enumerate(cfg.get('TRE', [4, 4, 4, 4])):
        addq((True, 'head', HB - 1 + j), cnt)
    for j, cnt in enumerate(cfg.get('TRO', [4, 4, 4, 4])):
        addq((False, 'head', HB - 1 + j), cnt)
    for j in range(0, 8 * WOQ - 1, cfg.get('WOSTEP', 2)):
        addq((True, 'woq', j), 1)
    addq((True, 'woq', 8 * WOQ - 1), cfg.get('ENDE', 5))
    rest = NC * UF * MPC - sum(qk_slots.values())
    ndot = cfg.get('NDOT', 3 * HB - 3)
    for i in range(rest):
        addq((False, 'dot', (i * ndot) // rest), 1)
    op_slots = {}
    for key in cfg.get('OPS', [(1, 'head', 31), (1, 'head', 32), (1, 'head', 33), (1, 'woq', 15), (1, 'woq', 31),
                               (0, 'dot', 11), (0, 'dot', 23), (0, 'dot', 35), (0, 'dot', 47), (0, 'dot', 59),
                               (0, 'dot', 71), (0, 'dot', 83), (0, 'head', 31), (0, 'head', 32), (0, 'head', 33),
                               (0, 'head', 34)]):
        key = (bool(key[0]), key[1], key[2])
        op_slots[key] = op_slots.get(key, 0) + 1
    assert sum(op_slots.values()) == 2 * OB // 32 and rest >= 0 and len(QAT) == QPI and RPI % 4 == 0

    def kernel(x_hbm, wq_hbm, wkt_hbm, wvt_hbm, wo_hbm, mem0_hbm, bq_hbm, bk_hbm, bv_hbm, bo_hbm, gw_hbm,
               out_hbm,
               x_v, wq_v, wo_v, wkv_v, mem0_v, gw_v, raw_v, wp_v, bo_v, qt_v, k_v, vt_v, sa_v, sb_v, o_v, b_v,
               sq_v, skv_v, ob_v, g_v,
               xsem, wqsem, wsem, bosem, wosem, osem):
        sbuf = (sa_v, sb_v)

        def x_copy(i):
            return pltpu.make_async_copy(x_hbm.at[pl.ds(i * XB, XB)], x_v.at[pl.ds(i * XB, XB)], xsem.at[i])

        def col_copies(src, dst, sem):
            return [pltpu.make_async_copy(src.at[:, pl.ds(n * 128, 128)], dst.at[n], sem.at[n]) for n in range(8)]

        def out_copy(i, slot):
            return pltpu.make_async_copy(ob_v.at[slot], out_hbm.at[pl.ds(i * OB, OB)], osem.at[slot])

        wq_copies = col_copies(wq_hbm, wq_v, wqsem)
        wo_copies = col_copies(wo_hbm, wo_v, wosem)
        bo_copies = col_copies(bo_hbm, bo_v, bosem)
        raw_copies = [pltpu.make_async_copy(src, raw_v.at[m], wsem.at[m])
                      for m, src in enumerate((bq_hbm, bk_hbm, bv_hbm))]
        wk_copy = pltpu.make_async_copy(wkt_hbm, wkv_v.at[pl.ds(0, DA)], wsem.at[3])
        wv_copy = pltpu.make_async_copy(wvt_hbm, wkv_v.at[pl.ds(DA, DA)], wsem.at[4])
        mem_copy = pltpu.make_async_copy(mem0_hbm, mem0_v, wsem.at[5])
        gw_copy = pltpu.make_async_copy(gw_hbm, gw_v, wsem.at[6])

        def kv_proj(rb):
            xb = x_v[rb * XB:(rb + 1) * XB, :]
            kvt = lax.dot_general(wkv_v[...], xb, NT, preferred_element_type=F32)
            k_v[rb * XB:(rb + 1) * XB, :] = kvt[:DA].T.astype(BF)
            for t in range(XB // 128):
                vt_v[rb * (XB // 128) + t] = kvt[DA:2 * DA, t * 128:(t + 1) * 128].astype(BF)

        def q_piece(tile, n, rows=128):
            r0 = tile * 128 if isinstance(tile, int) else pl.multiple_of(tile * 128, 128)
            c0 = n * 128 if isinstance(n, int) else pl.multiple_of(n * 128, 128)
            q = jnp.dot(x_v[pl.ds(r0, rows), :], wq_v[n], preferred_element_type=F32) * SCALE_A
            for t in range(rows // 128):
                qt_v[tile + t, pl.ds(c0, 128), :] = q[t * 128:(t + 1) * 128].T.astype(BF)

        def load_q(u):
            u = jnp.minimum(u, NUNITS - 1)
            base = pl.multiple_of(lax.shift_right_logical(u, 4) * 128, 128)
            return jnp.concatenate(
                [qt_v[u & 15, pl.ds(base + DA * j, DA), :] for j in range(4)], axis=1)

        def qk_rows(qt, s_ref, r0, rows, m8):
            sn = jnp.dot(k_v[r0:r0 + rows, :], qt, preferred_element_type=F32)
            s_ref[r0:r0 + rows, :] = sn
            for g in range(rows // 8):
                t = sn[g * 8:(g + 1) * 8]
                m8 = t if m8 is None else jnp.maximum(m8, t)
            return m8

        def pv_chunk(s_ref, c, me, l8, acc, ag):
            p = jnp.exp2(s_ref[c * 128:(c + 1) * 128, :].reshape(16, 8, 512) - me[None])
            for g in reversed(range(16)):
                l8 = p[g] if l8 is None else l8 + p[g]
                if g == ag:
                    anchor = l8
            pv = jnp.dot(vt_v[c], p.reshape(128, 512).astype(BF), preferred_element_type=F32)
            return l8, (pv if acc is None else acc + pv), anchor

        def finalize(u, acc, l8):
            u = jnp.maximum(u, 0)
            o = acc * pl.reciprocal(jnp.sum(l8, axis=0, keepdims=True), approx=True)
            ot = jnp.concatenate([o[:, j * 128:(j + 1) * 128] for j in range(4)], axis=0).T
            o_v[lax.shift_right_logical(u, 4), pl.ds(pl.multiple_of((u & 15) * 128, 128), 128), :] = ot.astype(BF)
            return ot[120:128]

        def a_tasks(u0, st):
            qts = [load_q(u0 + 1 + j) for j in range(UA + 1)]
            st.anchor, st.hist = None, []

            def task(k, c):
                if c == 0:
                    st.mc8 = jnp.broadcast_to(st.m, (8, 512))
                    st.l8, st.acc = None, None
                cn = c + SKEW
                if cn < NC:
                    st.m8 = qk_rows(qts[k], sbuf[(k + 1) % 2], cn * 128, 128, st.m8)
                    if cn == NC - 1:
                        st.mnext = jnp.max(st.m8, axis=0, keepdims=True)
                else:
                    st.m8 = qk_rows(qts[k + 1], sbuf[k % 2], (cn - NC) * 128, 128, None if cn == NC else st.m8)
                st.hist.append(st.m8)
                me = st.mc8
                if st.anchor is not None:
                    me = me + st.anchor * 0.0
                if len(st.hist) > LAGM:
                    me = me + st.hist[-1 - LAGM] * 0.0
                st.l8, st.acc, st.anchor = pv_chunk(sbuf[k % 2], c, me, st.l8, st.acc, AG)
                if c == FIN:
                    finalize(u0 + k - 1, st.pacc, st.pl8 + st.l8 * 0.0)
                if c == NC - 1:
                    st.pacc, st.pl8, st.m = st.acc, st.l8, st.mnext
            return [(lambda k=k, c=c: task(k, c)) for k in range(UA) for c in range(NC)]

        def relayout(sub, half, par, anchor):
            m = lax.shift_right_logical(sub, 8)
            i = lax.shift_right_logical(sub, 2) & 63
            msk = pltpu.bitcast(anchor[:, :128] * 0.0, U32) | jnp.uint32(0xFFFF0000 if par else 0xFFFF)
            w = raw_v[m, pl.ds(pl.multiple_of(i * 16, 16), 16), half * 16:(half + 1) * 16, :]
            outs = []
            for t in range(8):
                a = pltpu.bitcast(w[2 * t], U32)
                b = pltpu.bitcast(w[2 * t + 1], U32)
                outs.append(((a >> 16) | (b & msk)) if par else ((a & msk) | (b << 16)))
            tr = jnp.swapaxes(jnp.stack(outs), 0, 1)
            for j in range(8):
                wp_v[m, 16 * half + 2 * j + par, pl.ds(pl.multiple_of(i * 8, 8), 8), :] = tr[j]

        def gate_block(r0, rows, anchor):
            gw = gw_v[...].astype(F32)
            xg = jnp.concatenate([anchor[:, :128] * 0.0] * (rows // 8), axis=0)
            for g in range(8):
                xg = xg + x_v[pl.ds(r0, rows), g * 128:(g + 1) * 128].astype(F32) * gw[g:g + 1, :]
            gt = jnp.broadcast_to(jax.nn.sigmoid(jnp.sum(xg, axis=-1, keepdims=True)), (rows, 128))
            g_v[pl.ds(r0, rows), :] = gt
            return jnp.sum(gt.reshape(rows // 8, 8, 128), axis=0)

        def out_piece(r0, rows, n, slot, off):
            ol = jnp.concatenate([o_v[g, pl.ds(r0, rows), :] for g in range(8)], axis=1)
            a = jnp.dot(ol, wo_v[n], preferred_element_type=F32)
            g_ = g_v[pl.ds(r0, rows), :]
            res = g_ * a + (1.0 - g_) * b_v[pl.ds(r0, rows), n * 128:(n + 1) * 128]
            ob_v[slot, off:off + rows, n * 128:(n + 1) * 128] = res.astype(BF)
            return res

        wk_copy.start()
        wv_copy.start()
        gw_copy.start()
        x_copy(0).start()
        wk_copy.wait()
        wv_copy.wait()
        gw_copy.wait()
        for c in wq_copies[:NPG]:
            c.start()
        with jax.named_scope('P1_proj'):
            x_copy(0).wait()
            for i in range(1, NXB):
                x_copy(i).start()
            kv_proj(0)
            for c in wq_copies[:NPG]:
                c.wait()
            for rb in range(NXB):
                if rb in XWAIT:
                    for i in range(rb, XWAIT[rb]):
                        x_copy(i).wait()
                    if XWAIT[rb] == NXB:
                        for c in wq_copies[NPG:] + raw_copies + bo_copies + wo_copies + [mem_copy]:
                            c.start()
                if rb:
                    kv_proj(rb)
                for n in range(NPG):
                    q_piece(rb * (XB // 128), n, XB)

        m8 = None
        qt0 = load_q(0)
        for c in range(NC):
            m8 = qk_rows(qt0, sa_v, c * 128, 128, m8)
        m_init = jnp.max(m8, axis=0, keepdims=True)
        m8 = None
        qt1 = load_q(1)
        for c in range(SKEW):
            m8 = qk_rows(qt1, sb_v, c * 128, 128, m8)
        carry_a = (m_init, m8, jnp.zeros((DA, 512), F32), jnp.ones((8, 512), F32))

        def sa_body(it, carry):
            st = _State()
            st.m, st.m8, st.pacc, st.pl8 = carry
            for task in a_tasks(it * UA, st):
                task()
            return st.m, st.m8, st.pacc, st.pl8

        def sb_body(it, carry):
            for m in range(3):
                @pl.when(it == (256 * m) // RPI)
                def _():
                    raw_copies[m].wait()

            @pl.when(it == 0)
            def _():
                for c in wq_copies[NPG:]:
                    c.wait()
            st = _State()
            st.m, st.m8, st.pacc, st.pl8 = carry
            tasks = a_tasks((NIT_A + it) * UA, st)
            qn = [0]

            def q_at(pos):
                for _ in range(QAT.count(pos)):
                    pq = it * QPI + qn[0]
                    qn[0] += 1
                    q_piece(pq & 15, NPG + lax.shift_right_logical(pq, 4))
            q_at(-1)
            for n, task in enumerate(tasks):
                task()
                for r in range(n * RPI // len(tasks), (n + 1) * RPI // len(tasks)):
                    relayout(it * RPI + r, (r >> 1) & 1, r & 1, st.anchor)
                q_at(n)
            return st.m, st.m8, st.pacc, st.pl8

        with jax.named_scope('P2a_attn'):
            carry_a = lax.fori_loop(0, NIT_A, sa_body, carry_a)
        with jax.named_scope('P2b_attn'):
            carry_a = lax.fori_loop(0, NIT_B, sb_body, carry_a)

        for c in bo_copies + wo_copies:
            c.wait()
        mem_copy.wait()

        r = lax.broadcasted_iota(jnp.int32, (32, 48), 0)
        cc = lax.broadcasted_iota(jnp.int32, (32, 48), 1)
        mask_e = (cc >= 40) | ((cc < 32) & ((cc <= r) | (r >= 24)))
        fill_e = jnp.where(cc < 32, MASKED, -jnp.inf)
        r = lax.broadcasted_iota(jnp.int32, (48, 80), 0)
        cc = lax.broadcasted_iota(jnp.int32, (48, 80), 1)
        kseg = jnp.where((cc < 32) | ((cc >= 64) & (cc < 72)), 1, 0)
        kpos = jnp.where(cc < 24, cc + 8, jnp.where(cc < 32, -1, jnp.where(cc < 64, cc - 32,
                                                                           jnp.where(cc < 72, cc - 64, -1))))
        qseg = jnp.where(r < 40, 1, 0)
        qpos = jnp.where(r < 24, r + 8, jnp.where(r < 32, 100, jnp.where(r < 40, r - 32, r - 16)))
        mask_o = (kseg == qseg) & (kpos <= qpos)
        fill_o = jnp.where(kseg == qseg, MASKED, -jnp.inf)
        if cfg.get('NOFILL', 0):
            fill_e = fill_o = -1e30

        def b_step(lhs, even, base, hook, zget):
            mask, fill, l2 = (mask_e, fill_e, L2E) if even else (mask_o, fill_o, L2O)
            qkv, ps, os_ = {}, {}, {}

            def proj(m, h):
                y = jnp.dot(lhs, pltpu.bitcast(wp_v[m, h], BF), preferred_element_type=F32)
                hook(even, 'dot', 3 * h + m)
                return y

            def do_qkv(h):
                q = proj(0, h) * SCALE_B
                k = proj(1, h).astype(BF)
                v = proj(2, h).astype(BF)
                z = zget()
                q0 = q[0:8] if z is None else q[0:8] + z
                if even:
                    sq_v[h] = jnp.concatenate([q[32:40], q[24:32]], axis=0).astype(BF)
                    skv_v[2 * h] = k
                    skv_v[2 * h + 1] = v
                    q = jnp.concatenate([q0, q[8:24], q[40:48]], axis=0).astype(BF)
                else:
                    q = jnp.concatenate([jnp.concatenate([q0, q[8:32]], axis=0).astype(BF), sq_v[h]], axis=0)
                    k = jnp.concatenate([k, skv_v[2 * h]], axis=0)
                    v = jnp.concatenate([v, skv_v[2 * h + 1]], axis=0)
                qkv[h] = (q, k, v)

            def do_s(h):
                q, k, _ = qkv[h]
                s = jnp.where(mask, lax.dot_general(q, k, NT, preferred_element_type=F32), fill)
                p = jnp.exp2(s - jnp.max(s, axis=-1, keepdims=True))
                l = jnp.sum(p, axis=-1, keepdims=True)
                ps[h] = (p * pl.reciprocal(l, approx=True)).astype(BF)

            def do_pv(h):
                o = jnp.dot(ps[h], qkv[h][2], preferred_element_type=F32)
                z = zget() if h == HB - 1 else None
                if z is not None:
                    o = jnp.concatenate([o[0:8] + z, o[8:]], axis=0)
                os_[h] = o.astype(BF)

            for h in range(HB + L1 + l2):
                if h < HB:
                    do_qkv(h)
                if 0 <= h - L1 < HB:
                    do_s(h - L1)
                if 0 <= h - L1 - l2 < HB:
                    do_pv(h - L1 - l2)
                hook(even, 'head', h)
            nq = WOQ if even else 1
            hq = HB // nq
            ols = [jnp.concatenate([os_[h] for h in range(j * hq, (j + 1) * hq)], axis=1) for j in range(nq)]
            ms = []
            for n in range(8):
                y = None
                for j in range(nq):
                    t = jnp.dot(ols[j], bo_v[n, j * hq * DB:(j + 1) * hq * DB, :], preferred_element_type=F32)
                    y = t if y is None else y + t
                    hook(even, 'woq', n * nq + j)
                cols = slice(n * 128, (n + 1) * 128)
                if even:
                    b_v[pl.ds(base, 24), cols] = y[0:24]
                else:
                    b_v[pl.ds(base + 40, 24), cols] = y[0:24]
                    b_v[pl.ds(base + 32, 8), cols] = y[32:40]
                    b_v[pl.ds(base + 24, 8), cols] = y[40:48]
                z = zget() if n >= 2 else None
                ms.append((y[24:32] if z is None else y[24:32] + z).astype(BF))
            return jnp.concatenate(ms, axis=1)

        def fused_body(t, carry, last=False):
            u0 = NU_S + t * UF
            base = t * 64 if last else pl.multiple_of(t * 64, 64)
            st = _State()
            st.pv, st.qk, st.op, st.prev, st.hist, st.used, st.mn, st.fin = 0, 0, 0, None, [], 0, [], []

            def pv_task():
                k, c = divmod(st.pv, NC)
                st.pv += 1
                if c == 0:
                    st.mc8 = jnp.broadcast_to(carry[1 + k], (8, 512))
                    st.l8, st.acc = None, None
                me = st.mc8 if st.prev is None else st.mc8 + st.prev * 0.0
                st.l8, st.acc, st.prev = pv_chunk(sbuf[k], c, me, st.l8, st.acc, 0)
                if c == NC - 1:
                    st.fin.append((FLAG, finalize(u0 + k, st.acc, st.l8)))

            def qk_piece():
                k, i = divmod(st.qk, NC * MPC)
                st.qk += 1
                assert st.pv > k * NC + (i * MK) // 128
                if i == 0:
                    st.qt = load_q(u0 + UF + k)
                st.m8 = qk_rows(st.qt, sbuf[k], i * MK, MK, None if i == 0 else st.m8)
                st.hist.append(st.m8)
                if i == NC * MPC - 1:
                    st.mn.append(jnp.max(st.m8, axis=0, keepdims=True))

            def hook(even, kind, idx):
                key = (even, kind, idx)
                if even and kind == 'head' and idx in GAT:
                    gr = 64 // len(GAT)
                    st.fin.append((FLAG, gate_block(base + GAT.index(idx) * gr, gr, st.prev)))
                for _ in range(pv_slots.get(key, 0)):
                    pv_task()
                if not last:
                    for _ in range(qk_slots.get(key, 0)):
                        qk_piece()
                else:
                    for _ in range(op_slots.get(key, 0)):
                        half, n = divmod(st.op, 8)
                        st.op += 1
                        res = out_piece(half * 128, 128, n, 0, half * 128)
                        st.hist.append(jnp.sum(res.reshape(16, 8, 128), axis=0))

            def zget():
                z = None
                if st.fin and st.fin[0][0] <= 0:
                    z = st.fin.pop(0)[1]
                st.fin = [(a - 1, b) for a, b in st.fin]
                n = len(st.hist) - (OLAG if last else ZLAG)
                if n > st.used:
                    vals = st.hist[st.used:n] if last else st.hist[n - 1:n]
                    st.used = n
                    for v in vals:
                        if not last:
                            v = (v[:, 0:128] + v[:, 128:256]) + (v[:, 256:384] + v[:, 384:512])
                        z = v if z is None else z + v
                return None if z is None else z * 0.0

            mem = b_step(jnp.concatenate([x_v[pl.ds(base, 40), :], carry[0]], axis=0), True, base, hook, zget)
            mem = b_step(jnp.concatenate([x_v[pl.ds(base + 40, 24), :], mem], axis=0), False, base, hook, zget)
            return (mem,) + tuple(st.mn)

        finalize(NU_S - 1, carry_a[2], carry_a[3])
        qtb = load_q(NU_S + 1)
        m8 = carry_a[1]
        for c in range(SKEW, NC):
            m8 = qk_rows(qtb, sb_v, c * 128, 128, m8)
        with jax.named_scope('P3_fused'):
            carry = lax.fori_loop(0, NPAIR - 1, fused_body,
                                  (mem0_v[...], carry_a[0], jnp.max(m8, axis=0, keepdims=True)))
        with jax.named_scope('P3_last'):
            fused_body(NPAIR - 1, carry, last=True)
        out_copy(0, 0).start()

        def epi_body(i, carry):
            slot = i & 1

            @pl.when(i >= 2)
            def _():
                out_copy(i - 2, slot).wait()
            for n in range(8):
                out_piece(pl.multiple_of(i * OB, OB), OB, n, slot, 0)
            out_copy(i, slot).start()
            return carry
        with jax.named_scope('P4_epi'):
            lax.fori_loop(1, S // OB, epi_body, 0)
        out_copy(S // OB - 2, 0).wait()
        out_copy(S // OB - 1, 1).wait()

    def fn(A_x, A_wq, A_wk, A_wv, A_wo, B_x, B_mem0, B_Wq, B_Wk, B_Wv, B_Wo, B_seg_len, gate_w):
        any_spec = pl.BlockSpec(memory_space=pl.ANY)
        out = pl.pallas_call(
            kernel,
            out_shape=jax.ShapeDtypeStruct((S, D), BF),
            in_specs=[any_spec] * 11,
            out_specs=any_spec,
            scratch_shapes=[
                pltpu.VMEM((S, D), BF),
                pltpu.VMEM((8, D, 128), BF),
                pltpu.VMEM((8, D, 128), BF),
                pltpu.VMEM((2 * DA, D), BF),
                pltpu.VMEM((8, D), BF),
                pltpu.VMEM((8, 128), BF),
                pltpu.VMEM((3, D, HB, DB), BF),
                pltpu.VMEM((3, HB, D // 2, DB), U32),
                pltpu.VMEM((8, HB * DB, 128), BF),
                pltpu.VMEM((NQT, D, 128), BF),
                pltpu.VMEM((S, DA), BF),
                pltpu.VMEM((NC, DA, 128), BF),
                pltpu.VMEM((S, 512), F32),
                pltpu.VMEM((S, 512), F32),
                pltpu.VMEM((8, S, 128), BF),
                pltpu.VMEM((S, D), F32),
                pltpu.VMEM((HB, 16, DB), BF),
                pltpu.VMEM((2 * HB, 48, DB), BF),
                pltpu.VMEM((2, OB, D), BF),
                pltpu.VMEM((S, 128), F32),
                pltpu.SemaphoreType.DMA((NXB,)),
                pltpu.SemaphoreType.DMA((8,)),
                pltpu.SemaphoreType.DMA((7,)),
                pltpu.SemaphoreType.DMA((8,)),
                pltpu.SemaphoreType.DMA((8,)),
                pltpu.SemaphoreType.DMA((2,)),
            ],
            compiler_params=pltpu.CompilerParams(vmem_limit_bytes=120 * 1024 * 1024),
        )(A_x.reshape(S, D), A_wq, A_wk.T, A_wv.T, A_wo, B_mem0.reshape(8, D), B_Wq, B_Wk, B_Wv,
          B_Wo.reshape(HB * DB, D), gate_w.reshape(8, 128))
        return out.reshape(1, S, D)
    return jax.jit(fn)


_FN = build({"UA": 8})


@jax.jit
def pallas_gated_mix__grouped_kv_mqa__memory_aug_recurrent_mem_tr__prompt_kernel(
    A_x: jax.Array,
    A_wq: jax.Array,
    A_wk: jax.Array,
    A_wv: jax.Array,
    A_wo: jax.Array,
    B_x: jax.Array,
    B_mem0: jax.Array,
    B_Wq: jax.Array,
    B_Wk: jax.Array,
    B_Wv: jax.Array,
    B_Wo: jax.Array,
    B_seg_len: jax.Array,
    gate_w: jax.Array,
):
    return _FN(A_x, A_wq, A_wk, A_wv, A_wo, B_x, B_mem0, B_Wq, B_Wk, B_Wv, B_Wo, B_seg_len, gate_w)
```

```python
import jax
import jax.numpy as jnp
import numpy as np
from jax import lax
import jax.experimental.pallas as pl
import jax.experimental.pallas.tpu as pltpu

BF = jnp.bfloat16
F32 = jnp.float32
U32 = jnp.uint32

S = 2048
D = 1024
HA, DA = 32, 32
HB, DB = 32, 128
LOG2E = 1.4426950408889634
SCALE_A = float(np.asarray(DA ** -0.5, dtype=BF)) * LOG2E
SCALE_B = float(np.asarray(DB ** -0.5, dtype=BF)) * LOG2E
MASKED = float(np.asarray(-1e9, dtype=BF)) * LOG2E

XB = 256
NXB = S // XB
NQT = S // 128
NUNITS = NQT * (HA // 4)
NC = S // 128
OB = 256
NPAIR = S // 64
NT = (((1,), (1,)), ((), ()))


class _State:
    pass


def build(cfg):
    UA = cfg.get('UA', 4)
    QPI = 2 * UA
    UF = 2
    NU_S = NUNITS - UF * NPAIR
    NPG = 2
    NIT_B = (8 - NPG) * NQT // QPI
    NIT_A = NU_S // UA - NIT_B
    RPI = 768 // NIT_B
    SKEW = cfg.get('SKEW', 2)
    AG = cfg.get('AG', 8)
    LAGM = cfg.get('LAGM', 2)
    FIN = cfg.get('FIN', 0)
    QAT = cfg.get('QAT', [-1, -1] + [NC * k + p for k in range(UA - 1) for p in (14, 15)])
    xw = cfg.get('XW', [1, 3, 5, 8])
    XWAIT = dict(zip(xw[:-1], xw[1:]))
    L1 = cfg.get('L1', 1)
    L2E, L2O = cfg.get('L2E', 3), cfg.get('L2O', 3)
    WOQ = cfg.get('WOQ', 4)
    MK = 32
    MPC = 128 // MK
    ZLAG, OLAG, FLAG = cfg.get('ZLAG', 4), cfg.get('OLAG', 1), cfg.get('FLAG', 2)
    GAT = cfg.get('GAT', [5, 9, 20, 24])
    PVD = cfg.get('PVD', 2)

    pv_slots = {(True, 'dot', 3 * h + PVD): 1 for h in range(NC * UF)}
    qk_slots = {}
    def addq(key, cnt):
        qk_slots[key] = qk_slots.get(key, 0) + cnt
    for j, cnt in enumerate(cfg.get('TRE', [4, 4, 4, 4])):
        addq((True, 'head', HB - 1 + j), cnt)
    for j, cnt in enumerate(cfg.get('TRO', [4, 4, 4, 4])):
        addq((False, 'head', HB - 1 + j), cnt)
    for j in range(0, 8 * WOQ - 1, cfg.get('WOSTEP', 2)):
        addq((True, 'woq', j), 1)
    addq((True, 'woq', 8 * WOQ - 1), cfg.get('ENDE', 5))
    rest = NC * UF * MPC - sum(qk_slots.values())
    ndot = cfg.get('NDOT', 3 * HB - 3)
    for i in range(rest):
        addq((False, 'dot', (i * ndot) // rest), 1)
    op_slots = {}
    for key in cfg.get('OPS', [(1, 'head', 31), (1, 'head', 32), (1, 'head', 33), (1, 'woq', 15), (1, 'woq', 31),
                               (0, 'dot', 11), (0, 'dot', 23), (0, 'dot', 35), (0, 'dot', 47), (0, 'dot', 59),
                               (0, 'dot', 71), (0, 'dot', 83), (0, 'head', 31), (0, 'head', 32), (0, 'head', 33),
                               (0, 'head', 34)]):
        key = (bool(key[0]), key[1], key[2])
        op_slots[key] = op_slots.get(key, 0) + 1
    assert sum(op_slots.values()) == 2 * OB // 32 and rest >= 0 and len(QAT) == QPI and RPI % 4 == 0

    def kernel(x_hbm, wq_hbm, wkt_hbm, wvt_hbm, wo_hbm, mem0_hbm, bq_hbm, bk_hbm, bv_hbm, bo_hbm, gw_hbm,
               out_hbm,
               x_v, wq_v, wo_v, wkv_v, mem0_v, gw_v, raw_v, wp_v, bo_v, qt_v, k_v, vt_v, sa_v, sb_v, o_v, b_v,
               sq_v, skv_v, ob_v, g_v,
               xsem, wqsem, wsem, bosem, wosem, osem):
        sbuf = (sa_v, sb_v)

        def x_copy(i):
            return pltpu.make_async_copy(x_hbm.at[pl.ds(i * XB, XB)], x_v.at[pl.ds(i * XB, XB)], xsem.at[i])

        def col_copies(src, dst, sem):
            return [pltpu.make_async_copy(src.at[:, pl.ds(n * 128, 128)], dst.at[n], sem.at[n]) for n in range(8)]

        def out_copy(i, slot):
            return pltpu.make_async_copy(ob_v.at[slot], out_hbm.at[pl.ds(i * OB, OB)], osem.at[slot])

        wq_copies = col_copies(wq_hbm, wq_v, wqsem)
        wo_copies = col_copies(wo_hbm, wo_v, wosem)
        bo_copies = col_copies(bo_hbm, bo_v, bosem)
        raw_copies = [pltpu.make_async_copy(src, raw_v.at[m], wsem.at[m])
                      for m, src in enumerate((bq_hbm, bk_hbm, bv_hbm))]
        wk_copy = pltpu.make_async_copy(wkt_hbm, wkv_v.at[pl.ds(0, DA)], wsem.at[3])
        wv_copy = pltpu.make_async_copy(wvt_hbm, wkv_v.at[pl.ds(DA, DA)], wsem.at[4])
        mem_copy = pltpu.make_async_copy(mem0_hbm, mem0_v, wsem.at[5])
        gw_copy = pltpu.make_async_copy(gw_hbm, gw_v, wsem.at[6])

        def kv_proj(rb):
            xb = x_v[rb * XB:(rb + 1) * XB, :]
            kvt = lax.dot_general(wkv_v[...], xb, NT, preferred_element_type=F32)
            k_v[rb * XB // 2:(rb + 1) * XB // 2, :] = pltpu.bitcast(kvt[:DA].T.astype(BF), U32)
            for t in range(XB // 128):
                vt_v[rb * (XB // 128) + t] = pltpu.bitcast(kvt[DA:2 * DA, t * 128:(t + 1) * 128].astype(BF), U32)

        def q_piece(tile, n, rows=128):
            r0 = tile * 128 if isinstance(tile, int) else pl.multiple_of(tile * 128, 128)
            c0 = n * 64 if isinstance(n, int) else pl.multiple_of(n * 64, 64)
            q = jnp.dot(x_v[pl.ds(r0, rows), :], wq_v[n], preferred_element_type=F32) * SCALE_A
            for t in range(rows // 128):
                qt_v[tile + t, pl.ds(c0, 64), :] = pltpu.bitcast(q[t * 128:(t + 1) * 128].T.astype(BF), U32)

        def load_q(u):
            u = jnp.minimum(u, NUNITS - 1)
            base = pl.multiple_of(lax.shift_right_logical(u, 4) * 64, 64)
            return pltpu.bitcast(jnp.concatenate(
                [qt_v[u & 15, pl.ds(base + 16 * j, 16), :] for j in range(4)], axis=1), BF)

        def qk_rows(qt, s_ref, r0, rows, m8):
            kk = pltpu.bitcast(k_v[r0 // 2:(r0 + rows) // 2, :], BF)
            sn = jnp.dot(kk, qt, preferred_element_type=F32)
            s_ref[r0:r0 + rows, :] = sn
            for g in range(rows // 8):
                t = sn[g * 8:(g + 1) * 8]
                m8 = t if m8 is None else jnp.maximum(m8, t)
            return m8

        def pv_chunk(s_ref, c, me, l8, acc, ag):
            p = jnp.exp2(s_ref[c * 128:(c + 1) * 128, :].reshape(16, 8, 512) - me[None])
            for g in reversed(range(16)):
                l8 = p[g] if l8 is None else l8 + p[g]
                if g == ag:
                    anchor = l8
            pv = jnp.dot(pltpu.bitcast(vt_v[c], BF), p.reshape(128, 512).astype(BF), preferred_element_type=F32)
            return l8, (pv if acc is None else acc + pv), anchor

        def finalize(u, acc, l8):
            u = jnp.maximum(u, 0)
            o = acc * pl.reciprocal(jnp.sum(l8, axis=0, keepdims=True), approx=True)
            ot = jnp.concatenate([o[:, j * 128:(j + 1) * 128] for j in range(4)], axis=0).T
            o_v[lax.shift_right_logical(u, 4), pl.ds(pl.multiple_of((u & 15) * 64, 64), 64), :] = (
                pltpu.bitcast(ot.astype(BF), U32))
            return ot[120:128]

        def a_tasks(u0, st):
            qts = [load_q(u0 + 1 + j) for j in range(UA + 1)]
            st.anchor, st.hist = None, []

            def task(k, c):
                if c == 0:
                    st.mc8 = jnp.broadcast_to(st.m, (8, 512))
                    st.l8, st.acc = None, None
                cn = c + SKEW
                if cn < NC:
                    st.m8 = qk_rows(qts[k], sbuf[(k + 1) % 2], cn * 128, 128, st.m8)
                    if cn == NC - 1:
                        st.mnext = jnp.max(st.m8, axis=0, keepdims=True)
                else:
                    st.m8 = qk_rows(qts[k + 1], sbuf[k % 2], (cn - NC) * 128, 128, None if cn == NC else st.m8)
                st.hist.append(st.m8)
                me = st.mc8
                if st.anchor is not None:
                    me = me + st.anchor * 0.0
                if len(st.hist) > LAGM:
                    me = me + st.hist[-1 - LAGM] * 0.0
                st.l8, st.acc, st.anchor = pv_chunk(sbuf[k % 2], c, me, st.l8, st.acc, AG)
                if c == FIN:
                    finalize(u0 + k - 1, st.pacc, st.pl8 + st.l8 * 0.0)
                if c == NC - 1:
                    st.pacc, st.pl8, st.m = st.acc, st.l8, st.mnext
            return [(lambda k=k, c=c: task(k, c)) for k in range(UA) for c in range(NC)]

        def relayout(sub, half, par, anchor):
            m = lax.shift_right_logical(sub, 8)
            i = lax.shift_right_logical(sub, 2) & 63
            msk = pltpu.bitcast(anchor[:, :128] * 0.0, U32) | jnp.uint32(0xFFFF0000 if par else 0xFFFF)
            w = raw_v[m, pl.ds(pl.multiple_of(i * 16, 16), 16), half * 16:(half + 1) * 16, :]
            outs = []
            for t in range(8):
                a = pltpu.bitcast(w[2 * t], U32)
                b = pltpu.bitcast(w[2 * t + 1], U32)
                outs.append(((a >> 16) | (b & msk)) if par else ((a & msk) | (b << 16)))
            tr = jnp.swapaxes(jnp.stack(outs), 0, 1)
            for j in range(8):
                wp_v[m, 16 * half + 2 * j + par, pl.ds(pl.multiple_of(i * 8, 8), 8), :] = tr[j]

        def gate_block(r0, rows, anchor):
            gw = gw_v[...].astype(F32)
            xg = jnp.concatenate([anchor[:, :128] * 0.0] * (rows // 8), axis=0)
            for g in range(8):
                xg = xg + x_v[pl.ds(r0, rows), g * 128:(g + 1) * 128].astype(F32) * gw[g:g + 1, :]
            gt = jnp.broadcast_to(jax.nn.sigmoid(jnp.sum(xg, axis=-1, keepdims=True)), (rows, 128))
            g_v[pl.ds(r0, rows), :] = gt
            return jnp.sum(gt.reshape(rows // 8, 8, 128), axis=0)

        def out_piece(r0, rows, n, slot, off):
            h0 = r0 // 2 if isinstance(r0, int) else pl.multiple_of(lax.shift_right_logical(r0, 1), rows // 2)
            ol = pltpu.bitcast(jnp.concatenate([o_v[g, pl.ds(h0, rows // 2), :] for g in range(8)], axis=1), BF)
            a = jnp.dot(ol, wo_v[n], preferred_element_type=F32)
            g_ = g_v[pl.ds(r0, rows), :]
            res = g_ * a + (1.0 - g_) * b_v[pl.ds(r0, rows), n * 128:(n + 1) * 128]
            ob_v[slot, off:off + rows, n * 128:(n + 1) * 128] = res.astype(BF)
            return res

        wk_copy.start()
        wv_copy.start()
        gw_copy.start()
        x_copy(0).start()
        wk_copy.wait()
        wv_copy.wait()
        gw_copy.wait()
        for c in wq_copies[:NPG]:
            c.start()
        with jax.named_scope('P1_proj'):
            x_copy(0).wait()
            for i in range(1, NXB):
                x_copy(i).start()
            kv_proj(0)
            for c in wq_copies[:NPG]:
                c.wait()
            for rb in range(NXB):
                if rb in XWAIT:
                    for i in range(rb, XWAIT[rb]):
                        x_copy(i).wait()
                    if XWAIT[rb] == NXB:
                        for c in wq_copies[NPG:] + raw_copies:
                            c.start()
                if rb:
                    kv_proj(rb)
                for n in range(NPG):
                    q_piece(rb * (XB // 128), n, XB)

        m8 = None
        qt0 = load_q(0)
        for c in range(NC):
            m8 = qk_rows(qt0, sa_v, c * 128, 128, m8)
        m_init = jnp.max(m8, axis=0, keepdims=True)
        m8 = None
        qt1 = load_q(1)
        for c in range(SKEW):
            m8 = qk_rows(qt1, sb_v, c * 128, 128, m8)
        carry_a = (m_init, m8, jnp.zeros((DA, 512), F32), jnp.ones((8, 512), F32))

        def sa_body(it, carry):
            st = _State()
            st.m, st.m8, st.pacc, st.pl8 = carry
            for task in a_tasks(it * UA, st):
                task()
            return st.m, st.m8, st.pacc, st.pl8

        def sb_body(it, carry):
            for m in range(3):
                @pl.when(it == (256 * m) // RPI)
                def _():
                    raw_copies[m].wait()

            @pl.when(it == 0)
            def _():
                for c in wq_copies[NPG:]:
                    c.wait()
                for c in bo_copies + wo_copies + [mem_copy]:
                    c.start()
            st = _State()
            st.m, st.m8, st.pacc, st.pl8 = carry
            tasks = a_tasks((NIT_A + it) * UA, st)
            qn = [0]

            def q_at(pos):
                for _ in range(QAT.count(pos)):
                    pq = it * QPI + qn[0]
                    qn[0] += 1
                    q_piece(pq & 15, NPG + lax.shift_right_logical(pq, 4))
            q_at(-1)
            for n, task in enumerate(tasks):
                task()
                for r in range(n * RPI // len(tasks), (n + 1) * RPI // len(tasks)):
                    relayout(it * RPI + r, (r >> 1) & 1, r & 1, st.anchor)
                q_at(n)
            return st.m, st.m8, st.pacc, st.pl8

        with jax.named_scope('P2a_attn'):
            carry_a = lax.fori_loop(0, NIT_A, sa_body, carry_a)
        with jax.named_scope('P2b_attn'):
            carry_a = lax.fori_loop(0, NIT_B, sb_body, carry_a)

        for c in bo_copies + wo_copies:
            c.wait()
        mem_copy.wait()

        r = lax.broadcasted_iota(jnp.int32, (32, 48), 0)
        cc = lax.broadcasted_iota(jnp.int32, (32, 48), 1)
        mask_e = (cc >= 40) | ((cc < 32) & ((cc <= r) | (r >= 24)))
        fill_e = jnp.where(cc < 32, MASKED, -jnp.inf)
        r = lax.broadcasted_iota(jnp.int32, (48, 80), 0)
        cc = lax.broadcasted_iota(jnp.int32, (48, 80), 1)
        kseg = jnp.where((cc < 32) | ((cc >= 64) & (cc < 72)), 1, 0)
        kpos = jnp.where(cc < 24, cc + 8, jnp.where(cc < 32, -1, jnp.where(cc < 64, cc - 32,
                                                                           jnp.where(cc < 72, cc - 64, -1))))
        qseg = jnp.where(r < 40, 1, 0)
        qpos = jnp.where(r < 24, r + 8, jnp.where(r < 32, 100, jnp.where(r < 40, r - 32, r - 16)))
        mask_o = (kseg == qseg) & (kpos <= qpos)
        fill_o = jnp.where(kseg == qseg, MASKED, -jnp.inf)
        if cfg.get('NOFILL', 0):
            fill_e = fill_o = -1e30

        def b_step(lhs, even, base, hook, zget):
            mask, fill, l2 = (mask_e, fill_e, L2E) if even else (mask_o, fill_o, L2O)
            qkv, ps, os_ = {}, {}, {}

            def proj(m, h):
                y = jnp.dot(lhs, pltpu.bitcast(wp_v[m, h], BF), preferred_element_type=F32)
                hook(even, 'dot', 3 * h + m)
                return y

            def do_qkv(h):
                q = proj(0, h) * SCALE_B
                k = proj(1, h).astype(BF)
                v = proj(2, h).astype(BF)
                z = zget()
                q0 = q[0:8] if z is None else q[0:8] + z
                if even:
                    sq_v[h] = pltpu.bitcast(jnp.concatenate([q[32:40], q[24:32]], axis=0).astype(BF), U32)
                    skv_v[2 * h] = pltpu.bitcast(k, U32)
                    skv_v[2 * h + 1] = pltpu.bitcast(v, U32)
                    q = jnp.concatenate([q0, q[8:24], q[40:48]], axis=0).astype(BF)
                else:
                    q = jnp.concatenate([jnp.concatenate([q0, q[8:32]], axis=0).astype(BF), pltpu.bitcast(sq_v[h], BF)], axis=0)
                    k = jnp.concatenate([k, pltpu.bitcast(skv_v[2 * h], BF)], axis=0)
                    v = jnp.concatenate([v, pltpu.bitcast(skv_v[2 * h + 1], BF)], axis=0)
                qkv[h] = (q, k, v)

            def do_s(h):
                q, k, _ = qkv[h]
                s = jnp.where(mask, lax.dot_general(q, k, NT, preferred_element_type=F32), fill)
                p = jnp.exp2(s - jnp.max(s, axis=-1, keepdims=True))
                l = jnp.sum(p, axis=-1, keepdims=True)
                ps[h] = (p * pl.reciprocal(l, approx=True)).astype(BF)

            def do_pv(h):
                o = jnp.dot(ps[h], qkv[h][2], preferred_element_type=F32)
                z = zget() if h == HB - 1 else None
                if z is not None:
                    o = jnp.concatenate([o[0:8] + z, o[8:]], axis=0)
                os_[h] = o.astype(BF)

            for h in range(HB + L1 + l2):
                if h < HB:
                    do_qkv(h)
                if 0 <= h - L1 < HB:
                    do_s(h - L1)
                if 0 <= h - L1 - l2 < HB:
                    do_pv(h - L1 - l2)
                hook(even, 'head', h)
            nq = WOQ if even else 1
            hq = HB // nq
            ols = [jnp.concatenate([os_[h] for h in range(j * hq, (j + 1) * hq)], axis=1) for j in range(nq)]
            ms = []
            for n in range(8):
                y = None
                for j in range(nq):
                    t = jnp.dot(ols[j], bo_v[n, j * hq * DB:(j + 1) * hq * DB, :], preferred_element_type=F32)
                    y = t if y is None else y + t
                    hook(even, 'woq', n * nq + j)
                cols = slice(n * 128, (n + 1) * 128)
                if even:
                    b_v[pl.ds(base, 24), cols] = y[0:24]
                else:
                    b_v[pl.ds(base + 40, 24), cols] = y[0:24]
                    b_v[pl.ds(base + 32, 8), cols] = y[32:40]
                    b_v[pl.ds(base + 24, 8), cols] = y[40:48]
                z = zget() if n >= 2 else None
                ms.append((y[24:32] if z is None else y[24:32] + z).astype(BF))
            return jnp.concatenate(ms, axis=1)

        def fused_body(t, carry, last=False):
            u0 = NU_S + t * UF
            base = t * 64 if last else pl.multiple_of(t * 64, 64)
            st = _State()
            st.pv, st.qk, st.op, st.prev, st.hist, st.used, st.mn, st.fin = 0, 0, 0, None, [], 0, [], []

            def pv_task():
                k, c = divmod(st.pv, NC)
                st.pv += 1
                if c == 0:
                    st.mc8 = jnp.broadcast_to(carry[1 + k], (8, 512))
                    st.l8, st.acc = None, None
                me = st.mc8 if st.prev is None else st.mc8 + st.prev * 0.0
                st.l8, st.acc, st.prev = pv_chunk(sbuf[k], c, me, st.l8, st.acc, 0)
                if c == NC - 1:
                    st.fin.append((FLAG, finalize(u0 + k, st.acc, st.l8)))

            def qk_piece():
                k, i = divmod(st.qk, NC * MPC)
                st.qk += 1
                assert st.pv > k * NC + (i * MK) // 128
                if i == 0:
                    st.qt = load_q(u0 + UF + k)
                st.m8 = qk_rows(st.qt, sbuf[k], i * MK, MK, None if i == 0 else st.m8)
                st.hist.append(st.m8)
                if i == NC * MPC - 1:
                    st.mn.append(jnp.max(st.m8, axis=0, keepdims=True))

            def hook(even, kind, idx):
                key = (even, kind, idx)
                if even and kind == 'head' and idx in GAT:
                    gr = 64 // len(GAT)
                    st.fin.append((FLAG, gate_block(base + GAT.index(idx) * gr, gr, st.prev)))
                for _ in range(pv_slots.get(key, 0)):
                    pv_task()
                if not last:
                    for _ in range(qk_slots.get(key, 0)):
                        qk_piece()
                else:
                    for _ in range(op_slots.get(key, 0)):
                        half, n = divmod(st.op, 8)
                        st.op += 1
                        res = out_piece(half * 128, 128, n, 0, half * 128)
                        st.hist.append(jnp.sum(res.reshape(16, 8, 128), axis=0))

            def zget():
                z = None
                if st.fin and st.fin[0][0] <= 0:
                    z = st.fin.pop(0)[1]
                st.fin = [(a - 1, b) for a, b in st.fin]
                n = len(st.hist) - (OLAG if last else ZLAG)
                if n > st.used:
                    vals = st.hist[st.used:n] if last else st.hist[n - 1:n]
                    st.used = n
                    for v in vals:
                        if not last:
                            v = (v[:, 0:128] + v[:, 128:256]) + (v[:, 256:384] + v[:, 384:512])
                        z = v if z is None else z + v
                return None if z is None else z * 0.0

            mem = b_step(jnp.concatenate([x_v[pl.ds(base, 40), :], carry[0]], axis=0), True, base, hook, zget)
            mem = b_step(jnp.concatenate([x_v[pl.ds(base + 40, 24), :], mem], axis=0), False, base, hook, zget)
            return (mem,) + tuple(st.mn)

        finalize(NU_S - 1, carry_a[2], carry_a[3])
        qtb = load_q(NU_S + 1)
        m8 = carry_a[1]
        for c in range(SKEW, NC):
            m8 = qk_rows(qtb, sb_v, c * 128, 128, m8)
        with jax.named_scope('P3_fused'):
            carry = lax.fori_loop(0, NPAIR - 1, fused_body,
                                  (mem0_v[...], carry_a[0], jnp.max(m8, axis=0, keepdims=True)))
        with jax.named_scope('P3_last'):
            fused_body(NPAIR - 1, carry, last=True)
        out_copy(0, 0).start()

        def epi_body(i, carry):
            slot = i & 1

            @pl.when(i >= 2)
            def _():
                out_copy(i - 2, slot).wait()
            for n in range(8):
                out_piece(pl.multiple_of(i * OB, OB), OB, n, slot, 0)
            out_copy(i, slot).start()
            return carry
        with jax.named_scope('P4_epi'):
            lax.fori_loop(1, S // OB, epi_body, 0)
        out_copy(S // OB - 2, 0).wait()
        out_copy(S // OB - 1, 1).wait()

    def fn(A_x, A_wq, A_wk, A_wv, A_wo, B_x, B_mem0, B_Wq, B_Wk, B_Wv, B_Wo, B_seg_len, gate_w):
        any_spec = pl.BlockSpec(memory_space=pl.ANY)
        out = pl.pallas_call(
            kernel,
            out_shape=jax.ShapeDtypeStruct((S, D), BF),
            in_specs=[any_spec] * 11,
            out_specs=any_spec,
            scratch_shapes=[
                pltpu.VMEM((S, D), BF),
                pltpu.VMEM((8, D, 128), BF),
                pltpu.VMEM((8, D, 128), BF),
                pltpu.VMEM((2 * DA, D), BF),
                pltpu.VMEM((8, D), BF),
                pltpu.VMEM((8, 128), BF),
                pltpu.VMEM((3, D, HB, DB), BF),
                pltpu.VMEM((3, HB, D // 2, DB), U32),
                pltpu.VMEM((8, HB * DB, 128), BF),
                pltpu.VMEM((NQT, D // 2, 128), U32),
                pltpu.VMEM((S // 2, DA), U32),
                pltpu.VMEM((NC, DA // 2, 128), U32),
                pltpu.VMEM((S, 512), F32),
                pltpu.VMEM((S, 512), F32),
                pltpu.VMEM((8, S // 2, 128), U32),
                pltpu.VMEM((S, D), F32),
                pltpu.VMEM((HB, 8, DB), U32),
                pltpu.VMEM((2 * HB, 24, DB), U32),
                pltpu.VMEM((2, OB, D), BF),
                pltpu.VMEM((S, 128), F32),
                pltpu.SemaphoreType.DMA((NXB,)),
                pltpu.SemaphoreType.DMA((8,)),
                pltpu.SemaphoreType.DMA((7,)),
                pltpu.SemaphoreType.DMA((8,)),
                pltpu.SemaphoreType.DMA((8,)),
                pltpu.SemaphoreType.DMA((2,)),
            ],
            compiler_params=pltpu.CompilerParams(vmem_limit_bytes=120 * 1024 * 1024),
        )(A_x.reshape(S, D), A_wq, A_wk.T, A_wv.T, A_wo, B_mem0.reshape(8, D), B_Wq, B_Wk, B_Wv,
          B_Wo.reshape(HB * DB, D), gate_w.reshape(8, 128))
        return out.reshape(1, S, D)
    return jax.jit(fn)


_FN = build({"UA": 8, "XW": [1, 2, 4, 6, 8]})


@jax.jit
def pallas_gated_mix__grouped_kv_mqa__memory_aug_recurrent_mem_tr__prompt_kernel(
    A_x: jax.Array,
    A_wq: jax.Array,
    A_wk: jax.Array,
    A_wv: jax.Array,
    A_wo: jax.Array,
    B_x: jax.Array,
    B_mem0: jax.Array,
    B_Wq: jax.Array,
    B_Wk: jax.Array,
    B_Wv: jax.Array,
    B_Wo: jax.Array,
    B_seg_len: jax.Array,
    gate_w: jax.Array,
):
    return _FN(A_x, A_wq, A_wk, A_wv, A_wo, B_x, B_mem0, B_Wq, B_Wk, B_Wv, B_Wo, B_seg_len, gate_w)
```

```python
import jax
import jax.numpy as jnp
import numpy as np
from jax import lax
import jax.experimental.pallas as pl
import jax.experimental.pallas.tpu as pltpu

BF = jnp.bfloat16
F32 = jnp.float32
U32 = jnp.uint32

S = 2048
D = 1024
HA, DA = 32, 32
HB, DB = 32, 128
LOG2E = 1.4426950408889634
SCALE_A = float(np.asarray(DA ** -0.5, dtype=BF)) * LOG2E
SCALE_B = float(np.asarray(DB ** -0.5, dtype=BF)) * LOG2E
MASKED = float(np.asarray(-1e9, dtype=BF)) * LOG2E

XB = 256
NXB = S // XB
NQT = S // 128
NUNITS = NQT * (HA // 4)
NC = S // 128
OB = 256
NPAIR = S // 64
NT = (((1,), (1,)), ((), ()))


class _State:
    pass


UA = 8
QPI = 2 * UA
UF = 2
NU_S = NUNITS - UF * NPAIR
NPG = 2
NIT_B = (8 - NPG) * NQT // QPI
NIT_A = NU_S // UA - NIT_B
RPI = 768 // NIT_B
SKEW = 2
AG, LAGM = 8, 2
QAT = [-1, -1] + [NC * k + p for k in range(UA - 1) for p in (14, 15)]
XWAIT = {1: 2, 2: 4, 4: 6, 6: 8}
L1, L2 = 1, 3
WOQ = 4
MK = 32
MPC = 128 // MK
ZLAG, OLAG, FLAG = 4, 1, 2
GAT = [5, 9, 20, 24]
NS = 4
LB = 2


def _slots():
    pv = {(True, 'dot', 3 * h + 2): 1 for h in range(NC * UF)}
    qk, op = {}, {}

    def add(d, key, cnt=1):
        d[key] = d.get(key, 0) + cnt
    ndot = 3 * HB - 3
    for j in range(4):
        add(qk, (True, 'head', HB - 1 + j), 4)
        add(qk, (False, 'head', HB - 1 + j), 4)
    for j in range(0, 8 * WOQ - 1, 2):
        add(qk, (True, 'woq', j))
    add(qk, (True, 'woq', 8 * WOQ - 1), 5)
    rest = NC * UF * MPC - sum(qk.values())
    for i in range(rest):
        add(qk, (False, 'dot', (i * ndot) // rest))
    for j in range(3):
        add(op, (True, 'head', HB - 1 + j))
    for j in range(4):
        add(op, (False, 'head', HB - 1 + j))
        add(op, (True, 'woq', (j + 1) * 2 * WOQ - 1))
    rest = LB * OB // 128 * 8 - sum(op.values())
    for i in range(rest):
        add(op, (False, 'dot', ((2 * i + 1) * ndot) // (2 * rest)))
    return pv, qk, op


PV_SLOTS, QK_SLOTS, OP_SLOTS = _slots()


def _kernel(x_hbm, wq_hbm, wkt_hbm, wvt_hbm, wo_hbm, mem0_hbm, bq_hbm, bk_hbm, bv_hbm, bo_hbm, gw_hbm,
            out_hbm,
            x_v, wq_v, wo_v, wkv_v, mem0_v, gw_v, raw_v, wp_v, bo_v, qt_v, k_v, vt_v, sa_v, sb_v, o_v, b_v,
            sq_v, skv_v, ob_v, g_v,
            xsem, wqsem, wsem, bosem, wosem, osem):
    sbuf = (sa_v, sb_v)

    def x_copy(i):
        return pltpu.make_async_copy(x_hbm.at[pl.ds(i * XB, XB)], x_v.at[pl.ds(i * XB, XB)], xsem.at[i])

    def col_copies(src, dst, sem):
        return [pltpu.make_async_copy(src.at[:, pl.ds(n * 128, 128)], dst.at[n], sem.at[n]) for n in range(8)]

    def out_copy(i, slot, j):
        cols = pl.ds(j * (D // NS), D // NS)
        return pltpu.make_async_copy(ob_v.at[slot, :, cols], out_hbm.at[pl.ds(i * OB, OB), cols],
                                     osem.at[slot * NS + j])

    wq_copies = col_copies(wq_hbm, wq_v, wqsem)
    wo_copies = col_copies(wo_hbm, wo_v, wosem)
    bo_copies = col_copies(bo_hbm, bo_v, bosem)
    raw_copies = [pltpu.make_async_copy(src, raw_v.at[m], wsem.at[m])
                  for m, src in enumerate((bq_hbm, bk_hbm, bv_hbm))]
    wk_copy = pltpu.make_async_copy(wkt_hbm, wkv_v.at[pl.ds(0, DA)], wsem.at[3])
    wv_copy = pltpu.make_async_copy(wvt_hbm, wkv_v.at[pl.ds(DA, DA)], wsem.at[4])
    mem_copy = pltpu.make_async_copy(mem0_hbm, mem0_v, wsem.at[5])
    gw_copy = pltpu.make_async_copy(gw_hbm, gw_v, wsem.at[6])

    def kv_proj(rb):
        xb = x_v[rb * XB:(rb + 1) * XB, :]
        kvt = lax.dot_general(wkv_v[...], xb, NT, preferred_element_type=F32)
        k_v[rb * XB // 2:(rb + 1) * XB // 2, :] = pltpu.bitcast(kvt[:DA].T.astype(BF), U32)
        for t in range(XB // 128):
            vt_v[rb * (XB // 128) + t] = pltpu.bitcast(kvt[DA:2 * DA, t * 128:(t + 1) * 128].astype(BF), U32)

    def q_piece(tile, n, rows=128):
        r0 = tile * 128 if isinstance(tile, int) else pl.multiple_of(tile * 128, 128)
        c0 = n * 64 if isinstance(n, int) else pl.multiple_of(n * 64, 64)
        q = jnp.dot(x_v[pl.ds(r0, rows), :], wq_v[n], preferred_element_type=F32) * SCALE_A
        for t in range(rows // 128):
            qt_v[tile + t, pl.ds(c0, 64), :] = pltpu.bitcast(q[t * 128:(t + 1) * 128].T.astype(BF), U32)

    def load_q(u):
        u = jnp.minimum(u, NUNITS - 1)
        base = pl.multiple_of(lax.shift_right_logical(u, 4) * 64, 64)
        return pltpu.bitcast(jnp.concatenate(
            [qt_v[u & 15, pl.ds(base + 16 * j, 16), :] for j in range(4)], axis=1), BF)

    def qk_rows(qt, s_ref, r0, rows, m8):
        kk = pltpu.bitcast(k_v[r0 // 2:(r0 + rows) // 2, :], BF)
        sn = jnp.dot(kk, qt, preferred_element_type=F32)
        s_ref[r0:r0 + rows, :] = sn
        for g in range(rows // 8):
            t = sn[g * 8:(g + 1) * 8]
            m8 = t if m8 is None else jnp.maximum(m8, t)
        return m8

    def pv_chunk(s_ref, c, me, l8, acc, ag):
        p = jnp.exp2(s_ref[c * 128:(c + 1) * 128, :].reshape(16, 8, 512) - me[None])
        for g in reversed(range(16)):
            l8 = p[g] if l8 is None else l8 + p[g]
            if g == ag:
                anchor = l8
        pv = jnp.dot(pltpu.bitcast(vt_v[c], BF), p.reshape(128, 512).astype(BF), preferred_element_type=F32)
        return l8, (pv if acc is None else acc + pv), anchor

    def finalize(u, acc, l8):
        u = jnp.maximum(u, 0)
        o = acc * pl.reciprocal(jnp.sum(l8, axis=0, keepdims=True), approx=True)
        ot = jnp.concatenate([o[:, j * 128:(j + 1) * 128] for j in range(4)], axis=0).T
        o_v[lax.shift_right_logical(u, 4), pl.ds(pl.multiple_of((u & 15) * 64, 64), 64), :] = (
            pltpu.bitcast(ot.astype(BF), U32))
        return ot[120:128]

    def a_tasks(u0, st):
        qts = [load_q(u0 + 1 + j) for j in range(UA + 1)]
        st.anchor, st.hist = None, []

        def task(k, c):
            if c == 0:
                st.mc8 = jnp.broadcast_to(st.m, (8, 512))
                st.l8, st.acc = None, None
            cn = c + SKEW
            if cn < NC:
                st.m8 = qk_rows(qts[k], sbuf[(k + 1) % 2], cn * 128, 128, st.m8)
                if cn == NC - 1:
                    st.mnext = jnp.max(st.m8, axis=0, keepdims=True)
            else:
                st.m8 = qk_rows(qts[k + 1], sbuf[k % 2], (cn - NC) * 128, 128, None if cn == NC else st.m8)
            st.hist.append(st.m8)
            me = st.mc8
            if st.anchor is not None:
                me = me + st.anchor * 0.0
            if len(st.hist) > LAGM:
                me = me + st.hist[-1 - LAGM] * 0.0
            st.l8, st.acc, st.anchor = pv_chunk(sbuf[k % 2], c, me, st.l8, st.acc, AG)
            if c == 0:
                finalize(u0 + k - 1, st.pacc, st.pl8 + st.l8 * 0.0)
            if c == NC - 1:
                st.pacc, st.pl8, st.m = st.acc, st.l8, st.mnext
        return [(lambda k=k, c=c: task(k, c)) for k in range(UA) for c in range(NC)]

    def relayout(sub, half, par, anchor):
        m = lax.shift_right_logical(sub, 8)
        i = lax.shift_right_logical(sub, 2) & 63
        msk = pltpu.bitcast(anchor[:, :128] * 0.0, U32) | jnp.uint32(0xFFFF0000 if par else 0xFFFF)
        w = raw_v[m, pl.ds(pl.multiple_of(i * 16, 16), 16), half * 16:(half + 1) * 16, :]
        outs = []
        for t in range(8):
            a = pltpu.bitcast(w[2 * t], U32)
            b = pltpu.bitcast(w[2 * t + 1], U32)
            outs.append(((a >> 16) | (b & msk)) if par else ((a & msk) | (b << 16)))
        tr = jnp.swapaxes(jnp.stack(outs), 0, 1)
        for j in range(8):
            wp_v[m, 16 * half + 2 * j + par, pl.ds(pl.multiple_of(i * 8, 8), 8), :] = tr[j]

    def gate_block(r0, rows, anchor):
        gw = gw_v[...].astype(F32)
        xg = jnp.concatenate([anchor[:, :128] * 0.0] * (rows // 8), axis=0)
        for g in range(8):
            xg = xg + x_v[pl.ds(r0, rows), g * 128:(g + 1) * 128].astype(F32) * gw[g:g + 1, :]
        gt = jnp.broadcast_to(jax.nn.sigmoid(jnp.sum(xg, axis=-1, keepdims=True)), (rows, 128))
        g_v[pl.ds(r0, rows), :] = gt
        return jnp.sum(gt.reshape(rows // 8, 8, 128), axis=0)

    def out_piece(r0, rows, n, slot, off):
        h0 = r0 // 2 if isinstance(r0, int) else pl.multiple_of(lax.shift_right_logical(r0, 1), rows // 2)
        ol = pltpu.bitcast(jnp.concatenate([o_v[g, pl.ds(h0, rows // 2), :] for g in range(8)], axis=1), BF)
        a = jnp.dot(ol, wo_v[n], preferred_element_type=F32)
        g_ = g_v[pl.ds(r0, rows), :]
        res = g_ * a + (1.0 - g_) * b_v[pl.ds(r0, rows), n * 128:(n + 1) * 128]
        ob_v[slot, off:off + rows, n * 128:(n + 1) * 128] = res.astype(BF)
        return res

    wk_copy.start()
    wv_copy.start()
    gw_copy.start()
    x_copy(0).start()
    wk_copy.wait()
    wv_copy.wait()
    gw_copy.wait()
    for c in wq_copies[:NPG]:
        c.start()
    with jax.named_scope('P1_proj'):
        x_copy(0).wait()
        for i in range(1, NXB):
            x_copy(i).start()
        kv_proj(0)
        for c in wq_copies[:NPG]:
            c.wait()
        for rb in range(NXB):
            if rb in XWAIT:
                for i in range(rb, XWAIT[rb]):
                    x_copy(i).wait()
                if XWAIT[rb] == NXB:
                    for c in wq_copies[NPG:] + raw_copies:
                        c.start()
            if rb:
                kv_proj(rb)
            for n in range(NPG):
                q_piece(rb * (XB // 128), n, XB)

    m8 = None
    qt0 = load_q(0)
    for c in range(NC):
        m8 = qk_rows(qt0, sa_v, c * 128, 128, m8)
    m_init = jnp.max(m8, axis=0, keepdims=True)
    m8 = None
    qt1 = load_q(1)
    for c in range(SKEW):
        m8 = qk_rows(qt1, sb_v, c * 128, 128, m8)
    carry_a = (m_init, m8, jnp.zeros((DA, 512), F32), jnp.ones((8, 512), F32))

    def sa_body(it, carry):
        st = _State()
        st.m, st.m8, st.pacc, st.pl8 = carry
        for task in a_tasks(it * UA, st):
            task()
        return st.m, st.m8, st.pacc, st.pl8

    def sb_body(it, carry):
        for m in range(3):
            @pl.when(it == (256 * m) // RPI)
            def _():
                raw_copies[m].wait()

        @pl.when(it == 0)
        def _():
            for c in wq_copies[NPG:]:
                c.wait()
            for c in bo_copies + wo_copies + [mem_copy]:
                c.start()
        st = _State()
        st.m, st.m8, st.pacc, st.pl8 = carry
        tasks = a_tasks((NIT_A + it) * UA, st)
        qn = [0]

        def q_at(pos):
            for _ in range(QAT.count(pos)):
                pq = it * QPI + qn[0]
                qn[0] += 1
                q_piece(pq & 15, NPG + lax.shift_right_logical(pq, 4))
        q_at(-1)
        for n, task in enumerate(tasks):
            task()
            for r in range(n * RPI // len(tasks), (n + 1) * RPI // len(tasks)):
                relayout(it * RPI + r, (r >> 1) & 1, r & 1, st.anchor)
            q_at(n)
        return st.m, st.m8, st.pacc, st.pl8

    with jax.named_scope('P2a_attn'):
        carry_a = lax.fori_loop(0, NIT_A, sa_body, carry_a)
    with jax.named_scope('P2b_attn'):
        carry_a = lax.fori_loop(0, NIT_B, sb_body, carry_a)

    for c in bo_copies + wo_copies:
        c.wait()
    mem_copy.wait()

    r = lax.broadcasted_iota(jnp.int32, (32, 48), 0)
    cc = lax.broadcasted_iota(jnp.int32, (32, 48), 1)
    mask_e = (cc >= 40) | ((cc < 32) & ((cc <= r) | (r >= 24)))
    fill_e = jnp.where(cc < 32, MASKED, -jnp.inf)
    r = lax.broadcasted_iota(jnp.int32, (48, 80), 0)
    cc = lax.broadcasted_iota(jnp.int32, (48, 80), 1)
    kseg = jnp.where((cc < 32) | ((cc >= 64) & (cc < 72)), 1, 0)
    kpos = jnp.where(cc < 24, cc + 8, jnp.where(cc < 32, -1, jnp.where(cc < 64, cc - 32,
                                                                       jnp.where(cc < 72, cc - 64, -1))))
    qseg = jnp.where(r < 40, 1, 0)
    qpos = jnp.where(r < 24, r + 8, jnp.where(r < 32, 100, jnp.where(r < 40, r - 32, r - 16)))
    mask_o = (kseg == qseg) & (kpos <= qpos)
    fill_o = jnp.where(kseg == qseg, MASKED, -jnp.inf)

    def b_step(lhs, even, base, hook, zget):
        mask, fill = (mask_e, fill_e) if even else (mask_o, fill_o)
        qkv, ps, os_ = {}, {}, {}

        def proj(m, h):
            y = jnp.dot(lhs, pltpu.bitcast(wp_v[m, h], BF), preferred_element_type=F32)
            hook(even, 'dot', 3 * h + m)
            return y

        def do_qkv(h):
            q = proj(0, h) * SCALE_B
            k = proj(1, h).astype(BF)
            v = proj(2, h).astype(BF)
            z = zget()
            q0 = q[0:8] if z is None else q[0:8] + z
            if even:
                sq_v[h] = pltpu.bitcast(jnp.concatenate([q[32:40], q[24:32]], axis=0).astype(BF), U32)
                skv_v[2 * h] = pltpu.bitcast(k, U32)
                skv_v[2 * h + 1] = pltpu.bitcast(v, U32)
                q = jnp.concatenate([q0, q[8:24], q[40:48]], axis=0).astype(BF)
            else:
                q = jnp.concatenate([jnp.concatenate([q0, q[8:32]], axis=0).astype(BF), pltpu.bitcast(sq_v[h], BF)], axis=0)
                k = jnp.concatenate([k, pltpu.bitcast(skv_v[2 * h], BF)], axis=0)
                v = jnp.concatenate([v, pltpu.bitcast(skv_v[2 * h + 1], BF)], axis=0)
            qkv[h] = (q, k, v)

        def do_s(h):
            q, k, _ = qkv[h]
            s = jnp.where(mask, lax.dot_general(q, k, NT, preferred_element_type=F32), fill)
            p = jnp.exp2(s - jnp.max(s, axis=-1, keepdims=True))
            l = jnp.sum(p, axis=-1, keepdims=True)
            ps[h] = (p * pl.reciprocal(l, approx=True)).astype(BF)

        def do_pv(h):
            o = jnp.dot(ps[h], qkv[h][2], preferred_element_type=F32)
            z = zget() if h == HB - 1 else None
            if z is not None:
                o = jnp.concatenate([o[0:8] + z, o[8:]], axis=0)
            os_[h] = o.astype(BF)

        for h in range(HB + L1 + L2):
            if h < HB:
                do_qkv(h)
            if 0 <= h - L1 < HB:
                do_s(h - L1)
            if 0 <= h - L1 - L2 < HB:
                do_pv(h - L1 - L2)
            hook(even, 'head', h)
        nq = WOQ if even else 1
        hq = HB // nq
        ols = [jnp.concatenate([os_[h] for h in range(j * hq, (j + 1) * hq)], axis=1) for j in range(nq)]
        ms = []
        for n in range(8):
            y = None
            for j in range(nq):
                t = jnp.dot(ols[j], bo_v[n, j * hq * DB:(j + 1) * hq * DB, :], preferred_element_type=F32)
                y = t if y is None else y + t
                hook(even, 'woq', n * nq + j)
            cols = slice(n * 128, (n + 1) * 128)
            if even:
                b_v[pl.ds(base, 24), cols] = y[0:24]
            else:
                b_v[pl.ds(base + 40, 24), cols] = y[0:24]
                b_v[pl.ds(base + 32, 8), cols] = y[32:40]
                b_v[pl.ds(base + 24, 8), cols] = y[40:48]
            z = zget() if n >= 2 else None
            ms.append((y[24:32] if z is None else y[24:32] + z).astype(BF))
        return jnp.concatenate(ms, axis=1)

    def fused_body(t, carry, last=False):
        u0 = NU_S + t * UF
        base = t * 64 if last else pl.multiple_of(t * 64, 64)
        st = _State()
        st.pv, st.qk, st.op, st.prev, st.hist, st.used, st.mn, st.fin = 0, 0, 0, None, [], 0, [], []

        def pv_task():
            k, c = divmod(st.pv, NC)
            st.pv += 1
            if c == 0:
                st.mc8 = jnp.broadcast_to(carry[1 + k], (8, 512))
                st.l8, st.acc = None, None
            me = st.mc8 if st.prev is None else st.mc8 + st.prev * 0.0
            st.l8, st.acc, st.prev = pv_chunk(sbuf[k], c, me, st.l8, st.acc, 0)
            if c == NC - 1:
                st.fin.append((FLAG, finalize(u0 + k, st.acc, st.l8)))

        def qk_piece():
            k, i = divmod(st.qk, NC * MPC)
            st.qk += 1
            assert st.pv > k * NC + (i * MK) // 128
            if i == 0:
                st.qt = load_q(u0 + UF + k)
            st.m8 = qk_rows(st.qt, sbuf[k], i * MK, MK, None if i == 0 else st.m8)
            st.hist.append(st.m8)
            if i == NC * MPC - 1:
                st.mn.append(jnp.max(st.m8, axis=0, keepdims=True))

        def hook(even, kind, idx):
            key = (even, kind, idx)
            if even and kind == 'head' and idx in GAT:
                gr = 64 // len(GAT)
                st.fin.append((FLAG, gate_block(base + GAT.index(idx) * gr, gr, st.prev)))
            for _ in range(PV_SLOTS.get(key, 0)):
                pv_task()
            if not last:
                for _ in range(QK_SLOTS.get(key, 0)):
                    qk_piece()
            else:
                for _ in range(OP_SLOTS.get(key, 0)):
                    part, n = divmod(st.op, 8)
                    st.op += 1
                    res = out_piece(part * 128, 128, n, part * 128 // OB, part * 128 % OB)
                    st.hist.append(jnp.sum(res.reshape(16, 8, 128), axis=0))

        def zget():
            z = None
            if st.fin and st.fin[0][0] <= 0:
                z = st.fin.pop(0)[1]
            st.fin = [(a - 1, b) for a, b in st.fin]
            n = len(st.hist) - (OLAG if last else ZLAG)
            if n > st.used:
                vals = st.hist[st.used:n] if last else st.hist[n - 1:n]
                st.used = n
                for v in vals:
                    if not last:
                        v = (v[:, 0:128] + v[:, 128:256]) + (v[:, 256:384] + v[:, 384:512])
                    z = v if z is None else z + v
            return None if z is None else z * 0.0

        mem = b_step(jnp.concatenate([x_v[pl.ds(base, 40), :], carry[0]], axis=0), True, base, hook, zget)
        mem = b_step(jnp.concatenate([x_v[pl.ds(base + 40, 24), :], mem], axis=0), False, base, hook, zget)
        return (mem,) + tuple(st.mn)

    finalize(NU_S - 1, carry_a[2], carry_a[3])
    qtb = load_q(NU_S + 1)
    m8 = carry_a[1]
    for c in range(SKEW, NC):
        m8 = qk_rows(qtb, sb_v, c * 128, 128, m8)
    with jax.named_scope('P3_fused'):
        carry = lax.fori_loop(0, NPAIR - 1, fused_body,
                              (mem0_v[...], carry_a[0], jnp.max(m8, axis=0, keepdims=True)))
    with jax.named_scope('P3_last'):
        fused_body(NPAIR - 1, carry, last=True)
    for i in range(LB):
        for j in range(NS):
            out_copy(i, i, j).start()

    def epi_body(i, carry):
        slot = i & 1

        @pl.when(i >= 2)
        def _():
            for j in range(NS):
                out_copy(i - 2, slot, j).wait()
        for n in range(8):
            out_piece(pl.multiple_of(i * OB, OB), OB, n, slot, 0)
            if (n + 1) % (8 // NS) == 0:
                out_copy(i, slot, n // (8 // NS)).start()
        return carry
    with jax.named_scope('P4_epi'):
        lax.fori_loop(LB, S // OB, epi_body, 0)
    for j in range(NS):
        out_copy(S // OB - 2, 0, j).wait()
        out_copy(S // OB - 1, 1, j).wait()


@jax.jit
def pallas_gated_mix__grouped_kv_mqa__memory_aug_recurrent_mem_tr__prompt_kernel(
    A_x: jax.Array,
    A_wq: jax.Array,
    A_wk: jax.Array,
    A_wv: jax.Array,
    A_wo: jax.Array,
    B_x: jax.Array,
    B_mem0: jax.Array,
    B_Wq: jax.Array,
    B_Wk: jax.Array,
    B_Wv: jax.Array,
    B_Wo: jax.Array,
    B_seg_len: jax.Array,
    gate_w: jax.Array,
):
    any_spec = pl.BlockSpec(memory_space=pl.ANY)
    out = pl.pallas_call(
        _kernel,
        out_shape=jax.ShapeDtypeStruct((S, D), BF),
        in_specs=[any_spec] * 11,
        out_specs=any_spec,
        scratch_shapes=[
            pltpu.VMEM((S, D), BF),
            pltpu.VMEM((8, D, 128), BF),
            pltpu.VMEM((8, D, 128), BF),
            pltpu.VMEM((2 * DA, D), BF),
            pltpu.VMEM((8, D), BF),
            pltpu.VMEM((8, 128), BF),
            pltpu.VMEM((3, D, HB, DB), BF),
            pltpu.VMEM((3, HB, D // 2, DB), U32),
            pltpu.VMEM((8, HB * DB, 128), BF),
            pltpu.VMEM((NQT, D // 2, 128), U32),
            pltpu.VMEM((S // 2, DA), U32),
            pltpu.VMEM((NC, DA // 2, 128), U32),
            pltpu.VMEM((S, 512), F32),
            pltpu.VMEM((S, 512), F32),
            pltpu.VMEM((8, S // 2, 128), U32),
            pltpu.VMEM((S, D), F32),
            pltpu.VMEM((HB, 8, DB), U32),
            pltpu.VMEM((2 * HB, 24, DB), U32),
            pltpu.VMEM((2, OB, D), BF),
            pltpu.VMEM((S, 128), F32),
            pltpu.SemaphoreType.DMA((NXB,)),
            pltpu.SemaphoreType.DMA((8,)),
            pltpu.SemaphoreType.DMA((7,)),
            pltpu.SemaphoreType.DMA((8,)),
            pltpu.SemaphoreType.DMA((8,)),
            pltpu.SemaphoreType.DMA((2 * NS,)),
        ],
        compiler_params=pltpu.CompilerParams(vmem_limit_bytes=120 * 1024 * 1024),
    )(A_x.reshape(S, D), A_wq, A_wk.T, A_wv.T, A_wo, B_mem0.reshape(8, D), B_Wq, B_Wk, B_Wv,
      B_Wo.reshape(HB * DB, D), gate_w.reshape(8, 128))
    return out.reshape(1, S, D)
```

```python
import jax
import jax.numpy as jnp
import numpy as np
from jax import lax
import jax.experimental.pallas as pl
import jax.experimental.pallas.tpu as pltpu

BF = jnp.bfloat16
F32 = jnp.float32
U32 = jnp.uint32

S = 2048
D = 1024
HA, DA = 32, 32
HB, DB = 32, 128
LOG2E = 1.4426950408889634
SCALE_A = float(np.asarray(DA ** -0.5, dtype=BF)) * LOG2E
SCALE_B = float(np.asarray(DB ** -0.5, dtype=BF)) * LOG2E
MASKED = float(np.asarray(-1e9, dtype=BF)) * LOG2E

XB = 256
NXB = S // XB
NQT = S // 128
NUNITS = NQT * (HA // 4)
NC = S // 128
OB = 512
NPAIR = S // 64
NT = (((1,), (1,)), ((), ()))


class _State:
    pass


UA = 8
QPI = 2 * UA
UF = 2
NU_S = NUNITS - UF * NPAIR
NPG = 2
NIT_B = (8 - NPG) * NQT // QPI
NIT_A = NU_S // UA - NIT_B
RPI = 768 // NIT_B
SKEW = 2
AG, LAGM = 6, 2
QAT = [-1, 0, 14] + [NC * k + 14 for k in range(1, UA - 1) for _ in range(2)] + [126]
XWAIT = {1: 2, 2: 3, 3: 5, 5: 8}
L1, L2 = 1, 3
WOQ = 4
MK = 32
MPC = 128 // MK
ZLAG, OLAG, FLAG = 4, 1, 1
GAT = [3, 11, 19, 27]
NS = 8
LB = 1


def _slots():
    pv = {(True, 'dot', 3 * h + 2): 1 for h in range(NC * UF)}
    qk, op = {}, {}

    def add(d, key, cnt=1):
        d[key] = d.get(key, 0) + cnt
    ndot = 3 * HB
    for j in range(4):
        add(qk, (True, 'head', HB - 1 + j), 4)
        add(qk, (False, 'head', HB - 1 + j), 4)
    for j in range(0, 8 * WOQ - 1, 4):
        add(qk, (True, 'woq', j))
    add(qk, (True, 'woq', 8 * WOQ - 1), 5)
    rest = NC * UF * MPC - sum(qk.values())
    for i in range(rest):
        add(qk, (False, 'dot', (i * ndot) // rest))
    for j in range(3):
        add(op, (True, 'head', HB - 1 + j))
    for j in range(4):
        add(op, (False, 'head', HB - 1 + j))
        add(op, (True, 'woq', (j + 1) * 2 * WOQ - 1))
    rest = LB * OB // 128 * 8 - sum(op.values())
    for i in range(rest):
        add(op, (False, 'dot', ((2 * i + 1) * ndot) // (2 * rest)))
    return pv, qk, op


PV_SLOTS, QK_SLOTS, OP_SLOTS = _slots()


def _kernel(x_hbm, wq_hbm, wkt_hbm, wvt_hbm, wo_hbm, mem0_hbm, bq_hbm, bk_hbm, bv_hbm, bo_hbm, gw_hbm,
            out_hbm,
            x_v, wq_v, wo_v, wkv_v, mem0_v, gw_v, raw_v, wp_v, bo_v, qt_v, k_v, vt_v, sa_v, sb_v, o_v, b_v,
            sq_v, skv_v, ob_v, g_v,
            xsem, wqsem, wsem, bosem, wosem, osem):
    sbuf = (sa_v, sb_v)

    def x_copy(i):
        return pltpu.make_async_copy(x_hbm.at[pl.ds(i * XB, XB)], x_v.at[pl.ds(i * XB, XB)], xsem.at[i])

    def col_copies(src, dst, sem):
        return [pltpu.make_async_copy(src.at[:, pl.ds(n * 128, 128)], dst.at[n], sem.at[n]) for n in range(8)]

    def out_copy(i, slot, j):
        cols = pl.ds(j * (D // NS), D // NS)
        return pltpu.make_async_copy(ob_v.at[slot, :, cols], out_hbm.at[pl.ds(i * OB, OB), cols],
                                     osem.at[slot * NS + j])

    wq_copies = col_copies(wq_hbm, wq_v, wqsem)
    wo_copies = col_copies(wo_hbm, wo_v, wosem)
    bo_copies = col_copies(bo_hbm, bo_v, bosem)
    raw_copies = [pltpu.make_async_copy(src, raw_v.at[m], wsem.at[m])
                  for m, src in enumerate((bq_hbm, bk_hbm, bv_hbm))]
    wk_copy = pltpu.make_async_copy(wkt_hbm, wkv_v.at[pl.ds(0, DA)], wsem.at[3])
    wv_copy = pltpu.make_async_copy(wvt_hbm, wkv_v.at[pl.ds(DA, DA)], wsem.at[4])
    mem_copy = pltpu.make_async_copy(mem0_hbm, mem0_v, wsem.at[5])
    gw_copy = pltpu.make_async_copy(gw_hbm, gw_v, wsem.at[6])

    def kv_proj(rb):
        xb = x_v[rb * XB:(rb + 1) * XB, :]
        kvt = lax.dot_general(wkv_v[...], xb, NT, preferred_element_type=F32)
        k_v[rb * XB // 2:(rb + 1) * XB // 2, :] = pltpu.bitcast(kvt[:DA].T.astype(BF), U32)
        for t in range(XB // 128):
            vt_v[rb * (XB // 128) + t] = pltpu.bitcast(kvt[DA:2 * DA, t * 128:(t + 1) * 128].astype(BF), U32)

    def q_piece(tile, n, rows=128):
        r0 = tile * 128 if isinstance(tile, int) else pl.multiple_of(tile * 128, 128)
        c0 = n * 64 if isinstance(n, int) else pl.multiple_of(n * 64, 64)
        q = jnp.dot(x_v[pl.ds(r0, rows), :], wq_v[n], preferred_element_type=F32) * SCALE_A
        for t in range(rows // 128):
            qt_v[tile + t, pl.ds(c0, 64), :] = pltpu.bitcast(q[t * 128:(t + 1) * 128].T.astype(BF), U32)

    def load_q(u):
        u = jnp.minimum(u, NUNITS - 1)
        base = pl.multiple_of(lax.shift_right_logical(u, 4) * 64, 64)
        return pltpu.bitcast(jnp.concatenate(
            [qt_v[u & 15, pl.ds(base + 16 * j, 16), :] for j in range(4)], axis=1), BF)

    def qk_rows(qt, s_ref, r0, rows, m8):
        kk = pltpu.bitcast(k_v[r0 // 2:(r0 + rows) // 2, :], BF)
        sn = jnp.dot(kk, qt, preferred_element_type=F32)
        s_ref[r0:r0 + rows, :] = sn
        for g in range(rows // 8):
            t = sn[g * 8:(g + 1) * 8]
            m8 = t if m8 is None else jnp.maximum(m8, t)
        return m8

    def pv_chunk(s_ref, c, me, l8, acc, ag):
        p = jnp.exp2(s_ref[c * 128:(c + 1) * 128, :].reshape(16, 8, 512) - me[None])
        for g in reversed(range(16)):
            l8 = p[g] if l8 is None else l8 + p[g]
            if g == ag:
                anchor = l8
        pv = jnp.dot(pltpu.bitcast(vt_v[c], BF), p.reshape(128, 512).astype(BF), preferred_element_type=F32)
        return l8, (pv if acc is None else acc + pv), anchor

    def finalize(u, acc, l8):
        u = jnp.maximum(u, 0)
        o = acc * pl.reciprocal(jnp.sum(l8, axis=0, keepdims=True), approx=True)
        ot = jnp.concatenate([o[:, j * 128:(j + 1) * 128] for j in range(4)], axis=0).T
        o_v[lax.shift_right_logical(u, 4), pl.ds(pl.multiple_of((u & 15) * 64, 64), 64), :] = (
            pltpu.bitcast(ot.astype(BF), U32))
        return ot[120:128]

    def a_tasks(u0, st):
        qts = [load_q(u0 + 1 + j) for j in range(UA + 1)]
        st.anchor, st.hist = None, []

        def task(k, c):
            if c == 0:
                st.mc8 = jnp.broadcast_to(st.m, (8, 512))
                st.l8, st.acc = None, None
            cn = c + SKEW
            if cn < NC:
                st.m8 = qk_rows(qts[k], sbuf[(k + 1) % 2], cn * 128, 128, st.m8)
                if cn == NC - 1:
                    st.mnext = jnp.max(st.m8, axis=0, keepdims=True)
            else:
                st.m8 = qk_rows(qts[k + 1], sbuf[k % 2], (cn - NC) * 128, 128, None if cn == NC else st.m8)
            st.hist.append(st.m8)
            me = st.mc8
            if st.anchor is not None:
                me = me + st.anchor * 0.0
            if len(st.hist) > LAGM:
                me = me + st.hist[-1 - LAGM] * 0.0
            st.l8, st.acc, st.anchor = pv_chunk(sbuf[k % 2], c, me, st.l8, st.acc, AG)
            if c == 0:
                finalize(u0 + k - 1, st.pacc, st.pl8 + st.l8 * 0.0)
            if c == NC - 1:
                st.pacc, st.pl8, st.m = st.acc, st.l8, st.mnext
        return [(lambda k=k, c=c: task(k, c)) for k in range(UA) for c in range(NC)]

    def relayout(sub, oct_, anchor):
        m = lax.shift_right_logical(sub, 8)
        i = lax.shift_right_logical(sub, 2) & 63
        z = pltpu.bitcast(anchor[:, :128] * 0.0, U32)
        lo, hi = z | jnp.uint32(0xFFFF), z | jnp.uint32(0xFFFF0000)
        w = raw_v[m, pl.ds(pl.multiple_of(i * 16, 16), 16), oct_ * 8:(oct_ + 1) * 8, :]
        row = lax.broadcasted_iota(jnp.int32, (8, 128), 0)
        ev, od = [], []
        for t in range(4):
            a = pltpu.bitcast(jnp.concatenate([w[2 * t], w[2 * t + 8]], axis=0), U32)
            b = pltpu.bitcast(jnp.concatenate([w[2 * t + 1], w[2 * t + 9]], axis=0), U32)
            ev.append((a & lo) | (b << 16))
            od.append((a >> 16) | (b & hi))
        for par, v in enumerate((ev, od)):
            for k in (2, 1):
                keep = (row & k) == 0
                nv = list(v)
                for t in range(4):
                    if t & k == 0:
                        nv[t] = jnp.where(keep, v[t], pltpu.roll(v[t + k], k, 0))
                        nv[t + k] = jnp.where(keep, pltpu.roll(v[t], 8 - k, 0), v[t + k])
                v = nv
            for j in range(4):
                wp_v[m, 8 * oct_ + 2 * j + par, pl.ds(pl.multiple_of(i * 8, 8), 8), :] = v[j]

    def gate_block(r0, rows, anchor):
        gw = gw_v[...].astype(F32)
        xg = jnp.concatenate([anchor[:, :128] * 0.0] * (rows // 8), axis=0)
        for g in range(8):
            xg = xg + x_v[pl.ds(r0, rows), g * 128:(g + 1) * 128].astype(F32) * gw[g:g + 1, :]
        gt = jnp.broadcast_to(jax.nn.sigmoid(jnp.sum(xg, axis=-1, keepdims=True)), (rows, 128))
        g_v[pl.ds(r0, rows), :] = gt
        return jnp.sum(gt.reshape(rows // 8, 8, 128), axis=0)

    def out_piece(r0, rows, n, slot, off):
        h0 = r0 // 2 if isinstance(r0, int) else pl.multiple_of(lax.shift_right_logical(r0, 1), rows // 2)
        ol = pltpu.bitcast(jnp.concatenate([o_v[g, pl.ds(h0, rows // 2), :] for g in range(8)], axis=1), BF)
        a = jnp.dot(ol, wo_v[n], preferred_element_type=F32)
        g_ = g_v[pl.ds(r0, rows), :]
        res = g_ * a + (1.0 - g_) * b_v[pl.ds(r0, rows), n * 128:(n + 1) * 128]
        ob_v[slot, off:off + rows, n * 128:(n + 1) * 128] = res.astype(BF)
        return res

    wk_copy.start()
    wv_copy.start()
    gw_copy.start()
    x_copy(0).start()
    wk_copy.wait()
    wv_copy.wait()
    gw_copy.wait()
    for c in wq_copies[:NPG]:
        c.start()
    with jax.named_scope('P1_proj'):
        x_copy(0).wait()
        for i in range(1, NXB):
            x_copy(i).start()
        kv_proj(0)
        for c in wq_copies[:NPG]:
            c.wait()
        m8, cdone = None, 0
        for rb in range(NXB):
            if rb in XWAIT:
                for i in range(rb, XWAIT[rb]):
                    x_copy(i).wait()
                if XWAIT[rb] == NXB:
                    for c in wq_copies[NPG:] + raw_copies:
                        c.start()
            if rb:
                kv_proj(rb)
            for n in range(NPG):
                q_piece(rb * (XB // 128), n, XB)
            if rb:
                if rb == 1:
                    qt0 = load_q(0)
                for c in range(cdone, 2 * rb + 2):
                    m8 = qk_rows(qt0, sa_v, c * 128, 128, m8)
                cdone = 2 * rb + 2
        m_init = jnp.max(m8, axis=0, keepdims=True)
        m8 = None
        qt1 = load_q(1)
        for c in range(SKEW):
            m8 = qk_rows(qt1, sb_v, c * 128, 128, m8)
    carry_a = (m_init, m8, jnp.zeros((DA, 512), F32), jnp.ones((8, 512), F32))

    def sa_body(it, carry):
        st = _State()
        st.m, st.m8, st.pacc, st.pl8 = carry
        for task in a_tasks(it * UA, st):
            task()
        return st.m, st.m8, st.pacc, st.pl8

    def sb_body(it, carry):
        for m in range(3):
            @pl.when(it == (256 * m) // RPI)
            def _():
                raw_copies[m].wait()

        @pl.when(it == 0)
        def _():
            for c in wq_copies[NPG:]:
                c.wait()
            for c in bo_copies + wo_copies + [mem_copy]:
                c.start()
        st = _State()
        st.m, st.m8, st.pacc, st.pl8 = carry
        tasks = a_tasks((NIT_A + it) * UA, st)
        qn = [0]

        def q_at(pos):
            for _ in range(QAT.count(pos)):
                pq = it * QPI + qn[0]
                qn[0] += 1
                q_piece(pq & 15, NPG + lax.shift_right_logical(pq, 4))
        q_at(-1)
        for n, task in enumerate(tasks):
            task()
            for r in range(n * RPI // len(tasks), (n + 1) * RPI // len(tasks)):
                relayout(it * RPI + r, r & 3, st.l8)
            q_at(n)
        return st.m, st.m8, st.pacc, st.pl8

    with jax.named_scope('P2a_attn'):
        carry_a = lax.fori_loop(0, NIT_A, sa_body, carry_a)
    with jax.named_scope('P2b_attn'):
        carry_a = lax.fori_loop(0, NIT_B, sb_body, carry_a)

    for c in bo_copies + wo_copies:
        c.wait()
    mem_copy.wait()

    r = lax.broadcasted_iota(jnp.int32, (32, 48), 0)
    cc = lax.broadcasted_iota(jnp.int32, (32, 48), 1)
    mask_e = (cc >= 40) | ((cc < 32) & ((cc <= r) | (r >= 24)))
    fill_e = jnp.where(cc < 32, MASKED, -jnp.inf)
    r = lax.broadcasted_iota(jnp.int32, (48, 80), 0)
    cc = lax.broadcasted_iota(jnp.int32, (48, 80), 1)
    kseg = jnp.where((cc < 32) | ((cc >= 64) & (cc < 72)), 1, 0)
    kpos = jnp.where(cc < 24, cc + 8, jnp.where(cc < 32, -1, jnp.where(cc < 64, cc - 32,
                                                                       jnp.where(cc < 72, cc - 64, -1))))
    qseg = jnp.where(r < 40, 1, 0)
    qpos = jnp.where(r < 24, r + 8, jnp.where(r < 32, 100, jnp.where(r < 40, r - 32, r - 16)))
    mask_o = (kseg == qseg) & (kpos <= qpos)
    fill_o = jnp.where(kseg == qseg, MASKED, -jnp.inf)

    def b_step(lhs, even, base, hook, zget):
        mask, fill = (mask_e, fill_e) if even else (mask_o, fill_o)
        qkv, ps, os_ = {}, {}, {}

        def proj(m, h):
            y = jnp.dot(lhs, pltpu.bitcast(wp_v[m, h], BF), preferred_element_type=F32)
            hook(even, 'dot', 3 * h + m)
            return y

        def do_qkv(h):
            q = proj(0, h) * SCALE_B
            k = proj(1, h).astype(BF)
            v = proj(2, h).astype(BF)
            z = zget()
            q0 = q[0:8] if z is None else q[0:8] + z
            if even:
                sq_v[h] = pltpu.bitcast(jnp.concatenate([q[32:40], q[24:32]], axis=0).astype(BF), U32)
                skv_v[2 * h] = pltpu.bitcast(k, U32)
                skv_v[2 * h + 1] = pltpu.bitcast(v, U32)
                q = jnp.concatenate([q0, q[8:24], q[40:48]], axis=0).astype(BF)
            else:
                q = jnp.concatenate([q0, q[8:32]], axis=0).astype(BF)
                q = jnp.concatenate([q, pltpu.bitcast(sq_v[h], BF)], axis=0)
                k = jnp.concatenate([k, pltpu.bitcast(skv_v[2 * h], BF)], axis=0)
                v = jnp.concatenate([v, pltpu.bitcast(skv_v[2 * h + 1], BF)], axis=0)
            qkv[h] = (q, k, v)

        def do_s(h):
            q, k, _ = qkv[h]
            s = jnp.where(mask, lax.dot_general(q, k, NT, preferred_element_type=F32), fill)
            p = jnp.exp2(s - jnp.max(s, axis=-1, keepdims=True))
            l = jnp.sum(p, axis=-1, keepdims=True)
            ps[h] = (p * pl.reciprocal(l, approx=True)).astype(BF)

        def do_pv(h):
            o = jnp.dot(ps[h], qkv[h][2], preferred_element_type=F32)
            z = zget() if h == HB - 1 else None
            if z is not None:
                o = jnp.concatenate([o[0:8] + z, o[8:]], axis=0)
            os_[h] = o.astype(BF)

        for h in range(HB + L1 + L2):
            if h < HB:
                do_qkv(h)
            if 0 <= h - L1 < HB:
                do_s(h - L1)
            if 0 <= h - L1 - L2 < HB:
                do_pv(h - L1 - L2)
            hook(even, 'head', h)
        nq = WOQ if even else 1
        hq = HB // nq
        ols = [jnp.concatenate([os_[h] for h in range(j * hq, (j + 1) * hq)], axis=1) for j in range(nq)]
        ms = []
        for n in range(8):
            y = None
            for j in range(nq):
                t = jnp.dot(ols[j], bo_v[n, j * hq * DB:(j + 1) * hq * DB, :], preferred_element_type=F32)
                y = t if y is None else y + t
                hook(even, 'woq', n * nq + j)
            cols = slice(n * 128, (n + 1) * 128)
            if even:
                b_v[pl.ds(base, 24), cols] = y[0:24]
            else:
                b_v[pl.ds(base + 40, 24), cols] = y[0:24]
                b_v[pl.ds(base + 32, 8), cols] = y[32:40]
                b_v[pl.ds(base + 24, 8), cols] = y[40:48]
            z = zget() if n >= 2 else None
            ms.append((y[24:32] if z is None else y[24:32] + z).astype(BF))
        return jnp.concatenate(ms, axis=1)

    def fused_body(t, carry, last=False):
        u0 = NU_S + t * UF
        base = t * 64 if last else pl.multiple_of(t * 64, 64)
        st = _State()
        st.pv, st.qk, st.op, st.prev, st.hist, st.used, st.mn, st.fin = 0, 0, 0, None, [], 0, [], []

        def pv_task():
            k, c = divmod(st.pv, NC)
            st.pv += 1
            if c == 0:
                st.mc8 = jnp.broadcast_to(carry[1 + k], (8, 512))
                st.l8, st.acc = None, None
            me = st.mc8 if st.prev is None else st.mc8 + st.prev * 0.0
            st.l8, st.acc, st.prev = pv_chunk(sbuf[k], c, me, st.l8, st.acc, 0)
            if c == NC - 1:
                st.fin.append((FLAG, finalize(u0 + k, st.acc, st.l8)))

        def qk_piece():
            k, i = divmod(st.qk, NC * MPC)
            st.qk += 1
            assert st.pv > k * NC + (i * MK) // 128
            if i == 0:
                st.qt = load_q(u0 + UF + k)
            st.m8 = qk_rows(st.qt, sbuf[k], i * MK, MK, None if i == 0 else st.m8)
            st.hist.append(st.m8)
            if i == NC * MPC - 1:
                st.mn.append(jnp.max(st.m8, axis=0, keepdims=True))

        def hook(even, kind, idx):
            key = (even, kind, idx)
            if even and kind == 'head' and idx in GAT:
                gr = 64 // len(GAT)
                st.fin.append((FLAG, gate_block(base + GAT.index(idx) * gr, gr, st.prev)))
            for _ in range(PV_SLOTS.get(key, 0)):
                pv_task()
            if not last:
                for _ in range(QK_SLOTS.get(key, 0)):
                    qk_piece()
            else:
                for _ in range(OP_SLOTS.get(key, 0)):
                    part, n = divmod(st.op, 8)
                    st.op += 1
                    res = out_piece(part * 128, 128, n, part * 128 // OB, part * 128 % OB)
                    st.hist.append(jnp.max(res.reshape(16, 8, 128), axis=0))

        def zget():
            z = None
            if st.fin and st.fin[0][0] <= 0:
                z = st.fin.pop(0)[1]
            st.fin = [(a - 1, b) for a, b in st.fin]
            n = len(st.hist) - (OLAG if last else ZLAG)
            if n > st.used:
                vals = st.hist[st.used:n] if last else st.hist[n - 1:n]
                st.used = n
                for v in vals:
                    if not last:
                        v = jnp.maximum(jnp.maximum(v[:, 0:128], v[:, 128:256]),
                                        jnp.maximum(v[:, 256:384], v[:, 384:512]))
                    z = v if z is None else jnp.maximum(z, v)
            return None if z is None else z * 0.0

        mem = b_step(jnp.concatenate([x_v[pl.ds(base, 40), :], carry[0]], axis=0), True, base, hook, zget)
        mem = b_step(jnp.concatenate([x_v[pl.ds(base + 40, 24), :], mem], axis=0), False, base, hook, zget)
        return (mem,) + tuple(st.mn)

    finalize(NU_S - 1, carry_a[2], carry_a[3])
    qtb = load_q(NU_S + 1)
    m8 = carry_a[1]
    for c in range(SKEW, NC):
        m8 = qk_rows(qtb, sb_v, c * 128, 128, m8)
    with jax.named_scope('P3_fused'):
        carry = lax.fori_loop(0, NPAIR - 1, fused_body,
                              (mem0_v[...], carry_a[0], jnp.max(m8, axis=0, keepdims=True)))
    with jax.named_scope('P3_last'):
        fused_body(NPAIR - 1, carry, last=True)
    for i in range(LB):
        for j in range(NS):
            out_copy(i, i, j).start()

    def epi_body(i, carry):
        slot = i & 1

        @pl.when(i >= 2)
        def _():
            for j in range(NS):
                out_copy(i - 2, slot, j).wait()
        for n in range(8):
            out_piece(pl.multiple_of(i * OB, OB), OB, n, slot, 0)
            if (n + 1) % (8 // NS) == 0:
                out_copy(i, slot, n // (8 // NS)).start()
        return carry
    with jax.named_scope('P4_epi'):
        lax.fori_loop(LB, S // OB, epi_body, 0)
    for j in range(NS):
        out_copy(S // OB - 2, 0, j).wait()
        out_copy(S // OB - 1, 1, j).wait()


@jax.jit
def pallas_gated_mix__grouped_kv_mqa__memory_aug_recurrent_mem_tr__prompt_kernel(
    A_x: jax.Array,
    A_wq: jax.Array,
    A_wk: jax.Array,
    A_wv: jax.Array,
    A_wo: jax.Array,
    B_x: jax.Array,
    B_mem0: jax.Array,
    B_Wq: jax.Array,
    B_Wk: jax.Array,
    B_Wv: jax.Array,
    B_Wo: jax.Array,
    B_seg_len: jax.Array,
    gate_w: jax.Array,
):
    any_spec = pl.BlockSpec(memory_space=pl.ANY)
    out = pl.pallas_call(
        _kernel,
        out_shape=jax.ShapeDtypeStruct((S, D), BF),
        in_specs=[any_spec] * 11,
        out_specs=any_spec,
        scratch_shapes=[
            pltpu.VMEM((S, D), BF),
            pltpu.VMEM((8, D, 128), BF),
            pltpu.VMEM((8, D, 128), BF),
            pltpu.VMEM((2 * DA, D), BF),
            pltpu.VMEM((8, D), BF),
            pltpu.VMEM((8, 128), BF),
            pltpu.VMEM((3, D, HB, DB), BF),
            pltpu.VMEM((3, HB, D // 2, DB), U32),
            pltpu.VMEM((8, HB * DB, 128), BF),
            pltpu.VMEM((NQT, D // 2, 128), U32),
            pltpu.VMEM((S // 2, DA), U32),
            pltpu.VMEM((NC, DA // 2, 128), U32),
            pltpu.VMEM((S, 512), F32),
            pltpu.VMEM((S, 512), F32),
            pltpu.VMEM((8, S // 2, 128), U32),
            pltpu.VMEM((S, D), F32),
            pltpu.VMEM((HB, 8, DB), U32),
            pltpu.VMEM((2 * HB, 24, DB), U32),
            pltpu.VMEM((2, OB, D), BF),
            pltpu.VMEM((S, 128), F32),
            pltpu.SemaphoreType.DMA((NXB,)),
            pltpu.SemaphoreType.DMA((8,)),
            pltpu.SemaphoreType.DMA((7,)),
            pltpu.SemaphoreType.DMA((8,)),
            pltpu.SemaphoreType.DMA((8,)),
            pltpu.SemaphoreType.DMA((2 * NS,)),
        ],
        compiler_params=pltpu.CompilerParams(vmem_limit_bytes=120 * 1024 * 1024),
    )(A_x.reshape(S, D), A_wq, A_wk.T, A_wv.T, A_wo, B_mem0.reshape(8, D), B_Wq, B_Wk, B_Wv,
      B_Wo.reshape(HB * DB, D), gate_w.reshape(8, 128))
    return out.reshape(1, S, D)
```
